```python
import jax
import jax.numpy as jnp

def _softmax(x, axis=-1):
    return jax.nn.softmax(x, axis=axis)
def _gelu(x):
    return jax.nn.gelu(x, approximate=True)
def _silu(x):
    return jax.nn.silu(x)
def _sigmoid(x):
    return jax.nn.sigmoid(x)
def _layernorm(x, axis=-1, eps=1e-5):
    m = jnp.mean(x, axis=axis, keepdims=True)
    v = jnp.var(x, axis=axis, keepdims=True)
    return (x - m) / jnp.sqrt(v + eps)
def _scatter_add(tgt, idx, src, axis=0):
    return tgt.at[idx].add(src)
def _segment_sum(src, seg, n):
    return jax.ops.segment_sum(src, seg, n)
class _Rng:
    def __init__(self, key):
        self._k = key
    def _next(self):
        self._k, sub = jax.random.split(self._k)
        return sub
    def normal(self, shape):
        return jax.random.normal(self._next(), shape, dtype=jnp.bfloat16)
    def randint(self, lo, hi, shape):
        return jax.random.randint(self._next(), shape, lo, hi, dtype=jnp.int32)
    def uniform(self, shape, lo=0.0, hi=1.0):
        return jax.random.uniform(self._next(), shape, jnp.bfloat16, lo, hi)
    def permutation(self, n):
        return jax.random.permutation(self._next(), n)


kernel_name = 'recurrent_scan__compressed_kv_cla__dense_activation_gelu__decode'

def setup_inputs():
    _rng = _Rng(jax.random.key(int.from_bytes(__import__("os").urandom(4), "little")))
    _w = (lambda a: (lambda t: t.astype(jnp.bfloat16) if jnp.issubdtype(t.dtype, jnp.floating) else t)(jnp.asarray(a)))
    def _A_setup():
        B, H, Sq, Sk, D, M = 2, 32, 1, 16384, 128, 512
        Dc = 4 * D
        return {
            "x": _w((lambda *s: _rng.normal(s) * 0.05)(B, Sq, M)),
            "c_kv": _w((lambda *s: _rng.normal(s) * 0.05)(B, Sk, Dc)),
            "w_q": _w((lambda *s: _rng.normal(s) * 0.05)(M, H, D) * (M ** -0.5)),
            "w_uk": _w((lambda *s: _rng.normal(s) * 0.05)(Dc, H, D) * (Dc ** -0.5)),
            "w_uv": _w((lambda *s: _rng.normal(s) * 0.05)(Dc, H, D) * (Dc ** -0.5)),
            "w_o": _w((lambda *s: _rng.normal(s) * 0.05)(H, D, M) * ((H * D) ** -0.5)),
        }
    _A_in = _A_setup()

    def _B_setup():
        B, S, D, F = 2, 1, 512, 1792
        return {
            "x": _w((lambda *s: _rng.normal(s) * 0.05)(B, S, D)),
            "w1": _w((lambda *s: _rng.normal(s) * 0.05)(D, F) * (D ** -0.5)),
            "b1": _w((lambda *s: _rng.normal(s) * 0.05)(F) * 0.01),
            "w2": _w((lambda *s: _rng.normal(s) * 0.05)(F, D) * (F ** -0.5)),
            "b2": _w((lambda *s: _rng.normal(s) * 0.05)(D) * 0.01),
        }
    _B_in = _B_setup()

    return {
        "A_x": _A_in["x"],
        "A_c_kv": _A_in["c_kv"],
        "A_w_q": _A_in["w_q"],
        "A_w_uk": _A_in["w_uk"],
        "A_w_uv": _A_in["w_uv"],
        "A_w_o": _A_in["w_o"],
        "B_x": _B_in["x"],
        "B_w1": _B_in["w1"],
        "B_b1": _B_in["b1"],
        "B_w2": _B_in["w2"],
        "B_b2": _B_in["b2"],
    }

def reference(A_x, A_c_kv, A_w_q, A_w_uk, A_w_uv, A_w_o, B_x, B_w1, B_b1, B_w2, B_b2):
    def _A_ref(x, c_kv, w_q, w_uk, w_uv, w_o):
        B, Sq, M = x.shape[0], x.shape[1], x.shape[2]
        Sk = c_kv.shape[1]
        H, D = w_q.shape[1], w_q.shape[2]
        q = jnp.einsum("bqm,mhd->bhqd", x, w_q)
        k = jnp.einsum("bkc,chd->bhkd", c_kv, w_uk)
        v = jnp.einsum("bkc,chd->bhkd", c_kv, w_uv)
        scores = jnp.einsum("bhqd,bhkd->bhqk", q, k) * (D ** -0.5)
        off = Sk - Sq
        qi = jnp.arange(Sq)[:, None]
        kj = jnp.arange(Sk)[None, :]
        cmask = kj <= (qi + off)
        scores = jnp.where(cmask[None, None], scores, -1e9)
        p = _softmax(scores, axis=-1)
        ctx = jnp.einsum("bhqk,bhkd->bhqd", p, v)
        return jnp.einsum("bhqd,hdm->bqm", ctx, w_o)

    def _B_ref(x, w1, b1, w2, b2):
        h = jnp.einsum("bsd,df->bsf", x, w1) + b1
        h = _gelu(h)
        return jnp.einsum("bsf,fd->bsd", h, w2) + b2

    x = A_x
    xn = _layernorm(x, axis=-1)
    s = _A_ref(xn, A_c_kv, A_w_q, A_w_uk, A_w_uv, A_w_o)
    g = _silu(_B_ref(xn, B_w1, B_b1, B_w2, B_b2))
    return x + s * g
```

```python
import contextlib
import jax
import jax.numpy as jnp
from jax import lax
import jax.experimental.pallas as pl
import jax.experimental.pallas.tpu as pltpu

F32 = jnp.float32
BF16 = jnp.bfloat16
B, H, SK, D, M, DC, F = 2, 32, 16384, 128, 512, 512, 1792
LOG2E = 1.4426950408889634
NT = (((1,), (1,)), ((), ()))
W_VIEW = (4, 128, H, D)
C_VIEW = (32, 1024, DC)
O_VIEW = (4, 8 * D, M)
HG = 16


def _loop(lo, hi, body):
    lax.fori_loop(lo, hi, lambda i, _: body(i), None)


def _rows8(v):
    return jnp.concatenate([v[:, j * 128:(j + 1) * 128] for j in range(M // 128)], axis=0)


def make(LEAD=26, VH=(15, 23, 31), SPLIT=7, CUTS=(0, 128, 224, 288, 336, 368, 384), PH1=0, PH2=0, DMA_ONLY=False, REP=0, TR=False,
         CI=(0, 60, 100, 120), CTH=(1, 0, 0), HEAD=(3,), IG=(0, 1, 1), FLAGS=None):
    mark = (lambda n: jax.named_scope('@' + n)) if TR else (lambda n: contextlib.nullcontext())
    CONT = 8 * len(VH)
    assert CUTS[-1] == CONT * 16
    GROUPS = (0, 8, 16, 24, 32)

    o_list = []
    for j in range(32):
        for half in range(2):
            row = half * 512 + j * 16
            n = sum(a * 8 + row // D not in VH for a in range(4))
            assert all(a * 8 + row // D not in VH for a in range(n))
            o_list += [(0, 1, row, 16, 0, M, 0, j // 8)] * (n > 0) + [(1, n - 1, row, 16, 0, M, 1, j // 8)] * (n > 1)
    for i in range(CONT):
        a, row = divmod(VH[i // 8] * D + i % 8 * 16, 1024)
        cut = lambda r: 4 + max(k for k, c in enumerate(CUTS) if c <= i * 16 + r)
        if i < CONT - SPLIT:
            o_list.append((a, 1, row, 16, 0, M, CTH[(i - (CONT - SPLIT)) % len(CTH)], cut(0)))
        else:
            o_list += [(a, 1, row + r, 8, c, 256, 1, cut(r)) for r in (0, 8) for c in (0, 256)]
    o_t1 = [d for d in o_list if d[6] == 1]
    o_prog, k = [], LEAD
    for d in o_list:
        if d[6] == 0:
            o_prog.append(d)
        elif k < len(o_t1):
            o_prog.append(o_t1[k]); k += 1

    def body(x_hbm, ckv_hbm, wq_hbm, wuk_hbm, wuv_hbm, wo_hbm, w1_hbm, b1_hbm, w2_hbm, b2_hbm, o_hbm,
             x_buf, b1_buf, b2_buf, c_buf, wq_buf, wuk_buf, wuv_buf, wo_buf, w1_buf, w2_buf,
             xs, t8, qa_ref, acc_ref, m_ref, l_ref, a_buf, e_buf, ctx_ref, mul_ref, o_buf,
             sem_w, sem_c, sem_o, sem_small):
        def fetch(src, dst, sem, queue):
            pltpu.make_async_copy(src, dst, sem).start(priority=queue)

        def wait_filled(buf, sem):
            pltpu.make_async_copy(buf, buf, sem).wait()

        def when(c, f):
            if isinstance(c, bool):
                c and f()
            else:
                pl.when(c)(f)

        def quad_w(j, i, q):
            p1, p2 = (j + PH1) & 63, (j + PH2) & 63
            if i == 0 and q == 0:
                fetch(w2_hbm.at[p2], w2_buf.at[p2], sem_w.at[4], 0)
                when(p2 < 48, lambda: fetch(w2_hbm.at[p2 + 64], w2_buf.at[p2 + 64], sem_w.at[4], 0))
            elif i == 0:
                fetch(w1_hbm.at[p1], w1_buf.at[p1], sem_w.at[3], 1)
            else:
                if i == 1 and q == 0:
                    when(p1 < 48, lambda: fetch(w1_hbm.at[p1 + 64], w1_buf.at[p1 + 64], sem_w.at[3], 0))
                hbm, buf = ((wuv_hbm, wuv_buf), (wuk_hbm, wuk_buf), (wq_hbm, wq_buf))[i - 1]
                idx = (pl.ds(q, 1 + 2 * q), pl.ds(j * 2, 2))
                fetch(hbm.at[idx], buf.at[idx], sem_w.at[3 - i], q)

        def quad_c(r, i, q):
            row = (r & 63) * 16
            row = row if isinstance(r, int) else pl.multiple_of(row, 16)
            fetch(ckv_hbm.at[pl.ds((r >> 6) * 16 + 4 * i + q, 1 + 2 * q), pl.ds(row, 16)],
                  c_buf.at[pl.ds(r * 16 + 4 * i + q, 1 + 2 * q)], sem_c.at[r >> 3], q)

        def desc_o(d):
            a, n, row, nr, col, nc, q, s = d
            idx = (pl.ds(a, n), pl.ds(row, nr), pl.ds(col, nc))
            fetch(wo_hbm.at[idx], wo_buf.at[idx], sem_o.at[s], q)

        def half(g, q):
            if g < 256:
                quad_w(g // 4, g % 4, q)
            elif g < 768:
                quad_c(g // 4 - 64, g % 4, q)
            else:
                desc_o(o_t1[g - 768])

        def issue(lo, hi):
            for g in range(lo, hi):
                half(g, 0)
                half(g + LEAD, 1)

        def issue_rounds(quad, lo, hi):
            def one(r):
                for i in range(4):
                    quad(r, i, 0)
                    quad(r + (i + LEAD) // 4, (i + LEAD) % 4, 1)
            _loop(lo, hi, one)

        def issue_o(k):
            with mark(f'io{k}'):
                for d in o_prog[CI[k]:(CI + (None,))[k + 1]]:
                    desc_o(d)

        x_copy = pltpu.make_async_copy(x_hbm, x_buf, sem_small.at[0])
        b1_copy = pltpu.make_async_copy(b1_hbm, b1_buf, sem_small.at[1])
        b2_copy = pltpu.make_async_copy(b2_hbm, b2_buf, sem_small.at[2])
        o_copy = pltpu.make_async_copy(o_buf, o_hbm, sem_small.at[0])
        t0 = 0
        for g in range(LEAD + 8):
            half(g, 1)
            if g in HEAD or (g >= LEAD - 1 and t0 <= g - LEAD + 1 and t0 < 8):
                half(t0, 0); t0 += 1
        assert t0 == 8
        for c in (x_copy, b1_copy, b2_copy):
            c.start()
        LR = -(-LEAD // 4)

        def wait_group(g):
            lo, hi = GROUPS[g], GROUPS[g + 1]
            n = sum(d[1] * d[3] for d in o_list if d[7] == g)
            wait_filled(wo_buf.at[0, pl.ds(0, n)], sem_o.at[g])

        def wait_cut(i):
            a, row = divmod(VH[CUTS[i] // D] * D + CUTS[i] % D, 1024)
            n = CUTS[i + 1] - CUTS[i]
            wait_filled(wo_buf.at[a, pl.ds(min(row, 1024 - n), n)], sem_o.at[4 + i])

        if DMA_ONLY:
            issue_rounds(quad_w, 2, 64 - LR)
            issue(256 - 4 * LR, 256)
            issue_rounds(quad_c, 0, 128 - LR)
            issue(768 - 4 * LR, 768)
            for c in (x_copy, b1_copy, b2_copy):
                c.wait()
            for i, v in enumerate((wq_buf, wuk_buf, wuv_buf, w1_buf, w2_buf)):
                wait_filled(v, sem_w.at[i])
            for k in range(len(CI)):
                issue_o(k)
            for i in range(16):
                wait_filled(c_buf.at[pl.ds(i * 128, 128)], sem_c.at[i])
            for g in range(len(GROUPS) - 1):
                wait_group(g)
            for i in range(len(CUTS) - 1):
                wait_cut(i)
            o_copy.start()
            o_copy.wait()
            return

        with mark('iA0'):
            issue_rounds(quad_w, 2, 16)
        x_copy.wait()
        x = x_buf[...].astype(F32)
        xc = x - jnp.mean(x, axis=-1, keepdims=True)
        var = jnp.mean(xc * xc, axis=-1, keepdims=True)
        xn = (xc * lax.rsqrt(var + 1e-5)).astype(BF16)
        xf = xn.astype(F32)
        for b in range(B):
            for j in range(M // 128):
                cols = slice(j * 128, (j + 1) * 128)
                xs[b, cols, :] = jnp.broadcast_to(xf[b:b + 1, cols], (128, 128)).T
        e_buf[...] = (lax.broadcasted_iota(jnp.int32, (128, 128 * HG), 1) // HG
                      == lax.broadcasted_iota(jnp.int32, (128, 128 * HG), 0)).astype(F32).astype(BF16)
        m_ref[...] = jnp.full((B * H, 128), -jnp.inf, F32)
        l_ref[...] = jnp.zeros((B * H, 128), F32)
        acc_ref[...] = jnp.zeros((B * H, DC), F32)
        with mark('iA1'):
            issue_rounds(quad_w, 16, 64 - LR)
            issue(256 - 4 * LR, 256)
            issue_rounds(quad_c, 0, 8)

        with mark('wq'):
            wait_filled(wq_buf, sem_w.at[0])

        def q_run(a, carry):
            def q_body(i, carry):
                q0, q1 = carry
                for u in range(8):
                    m = pl.ds(a * 128 + i * 8 + u, 1)
                    w = wq_buf[a, i * 8 + u].astype(F32)
                    q0 = q0 + xs[0, m, :] * w
                    q1 = q1 + xs[1, m, :] * w
                return q0, q1
            carry = lax.fori_loop(0, 16, q_body, carry)
            with mark('iq'):
                issue_rounds(quad_c, 8 + 2 * a, 10 + 2 * a)
            return carry

        q0, q1 = lax.fori_loop(0, 4, q_run, (jnp.zeros((H, D), F32), jnp.zeros((H, D), F32)))
        q = jnp.concatenate([q0, q1, jnp.zeros((128 - B * H, D), F32)], axis=0).astype(BF16)

        wait_filled(wuk_buf, sem_w.at[1])
        group = (lax.broadcasted_iota(jnp.int32, (16, 8, 128), 2) % H) // 8

        def qa_body(i):
            for u in range(8):
                w = wuk_buf[i, pl.ds(u * 16, 16)].reshape(16 * H, D)
                r = lax.dot_general(w, q, NT, preferred_element_type=F32).reshape(16, 4, 8, 128)
                v = jnp.where(group == 0, r[:, 0],
                              jnp.where(group == 1, r[:, 1], jnp.where(group == 2, r[:, 2], r[:, 3])))
                t8[pl.ds(pl.multiple_of((i * 8 + u) * 128, 128), 128), :] = v.reshape(128, 128)
            with mark('iqa'):
                issue_rounds(quad_c, 16 + 3 * i, 19 + 3 * i)

        _loop(0, 4, qa_body)
        sub = lax.broadcasted_iota(jnp.int32, (128, 128), 1) % 8
        for j in range(DC // 128):
            t = t8[pl.ds(j * 1024, 128, stride=8), :]
            for s in range(1, 8):
                t = jnp.where(sub == s, t8[pl.ds(j * 1024 + s, 128, stride=8), :], t)
            qa_ref[:, j * 128:(j + 1) * 128] = (t.T[:B * H] * (D ** -0.5 * LOG2E)).astype(BF16)
        with mark('it'):
            issue_rounds(quad_c, 28, 31)

        wait_filled(w1_buf, sem_w.at[3])
        wait_filled(w2_buf, sem_w.at[4])
        b1_copy.wait()
        b2_copy.wait()
        w1 = w1_buf[...].reshape(M // 8, F // 128, 8, 128)
        hid = jnp.concatenate([jnp.dot(xn, w1[:, n].reshape(M, 128), preferred_element_type=F32)
                               for n in range(F // 128)], axis=1)
        hid = jax.nn.gelu(hid + b1_buf[...].astype(F32).reshape(1, F), approximate=True).astype(BF16)
        with mark('if'):
            issue_rounds(quad_c, 31, 35)
        z = jnp.dot(hid, w2_buf[...].reshape(F, M), preferred_element_type=F32)
        z8 = _rows8(z + b2_buf[...].astype(F32).reshape(1, M))
        g8 = z8 * jax.nn.sigmoid(z8)
        x8 = _rows8(x)
        wait_filled(wuv_buf, sem_w.at[2])

        diag = (lax.broadcasted_iota(jnp.int32, (H, 128 * HG), 1) % HG
                == lax.broadcasted_iota(jnp.int32, (H, 128 * HG), 0) % HG)

        def expand(b, hrows):
            pc = (acc_ref[hrows, :] / l_ref[hrows, :][:, :1]).astype(BF16)
            for j in range(DC // 128):
                rep = jnp.dot(pc[:, j * 128:(j + 1) * 128], e_buf[...], preferred_element_type=F32)
                a = jnp.where(diag, rep, 0.0).astype(BF16)
                for hg in range(H // HG):
                    a_buf[hg, j, b] = a[hg * HG:(hg + 1) * HG]

        def block(i):
            lo = jnp.maximum(32 + 6 * i, 8 * i + 8)
            hi = jnp.maximum(38 + 6 * i, 8 * i + 16)
            with mark('ib'):
                issue_rounds(quad_c, jnp.maximum(lo, 35), jnp.minimum(hi, 128 - LR))
                pl.when(i == 14)(lambda: issue(768 - 4 * LR, 768))
                pl.when(i == 15)(lambda: issue_o(0))
            b = i >> 3
            keys = c_buf.at[pl.ds(i * 128, 128)]
            with mark('wc'):
                wait_filled(keys, sem_c.at[i])
            hrows = pl.ds(pl.multiple_of(b * H, H), H)
            c = keys[...].reshape(2048, DC)
            sc = lax.dot_general(qa_ref[hrows, :], c, NT, preferred_element_type=F32)
            m_prev = m_ref[hrows, :]
            m_new = jnp.maximum(m_prev, jnp.max(sc, axis=1, keepdims=True))
            p = jnp.exp2(sc - m_new[:, :1])
            alpha = jnp.exp2(m_prev - m_new)
            l_ref[hrows, :] = alpha * l_ref[hrows, :] + jnp.sum(p, axis=1, keepdims=True)
            m_ref[hrows, :] = m_new
            pv = jnp.dot(p.astype(BF16), c, preferred_element_type=F32)
            acc_ref[hrows, :] = acc_ref[hrows, :] * alpha[:, :1] + pv

            @pl.when((i & 7) == 7)
            def _():
                pl.when(i == 15)(lambda: issue_o(1))
                expand(b, hrows)

        _loop(0, 16, block)
        if IG[0]:
            issue_o(2)
        for hg in range(H // HG):
            ctx = jnp.zeros((B * HG, D), F32)
            for j in range(DC // 128):
                ctx = ctx + jnp.dot(a_buf[hg, j].reshape(B * HG, 128 * HG),
                                    wuv_buf[j, :, hg * HG:(hg + 1) * HG].reshape(128 * HG, D),
                                    preferred_element_type=F32)
            for b in range(B):
                ctx_ref[b * H + hg * HG:b * H + (hg + 1) * HG] = ctx[b * HG:(b + 1) * HG]
        if not IG[0]:
            issue_o(2)
        for b in range(B):
            for i, h in enumerate(VH):
                cb = ctx_ref[b * H + h:b * H + h + 1].astype(BF16).astype(F32)
                mul_ref[b, i * D:(i + 1) * D] = jnp.broadcast_to(cb, (128, 128)).T
        if IG[1]:
            issue_o(3)

        s = jnp.zeros((B, M), F32)
        for g in range(len(GROUPS) - 1):
            lo, hi = GROUPS[g] * 16, GROUPS[g + 1] * 16
            with mark(f'wo{g}'):
                wait_group(g)
            hs = [h for h in range(g, H, 4) if h not in VH]
            lhs = [ctx_ref[pl.ds(h, B, stride=H), :] for h in hs]
            rhs = [wo_buf[h // 8, h % 8 * D:(h % 8 + 1) * D] for h in hs]
            s = s + jnp.dot(jnp.concatenate(lhs, axis=1).astype(BF16), jnp.concatenate(rhs, axis=0),
                            preferred_element_type=F32)
            if g == IG[2] - 1 and not IG[1]:
                issue_o(3)
        base8 = x8 + _rows8(s) * g8

        part = [[None] * (M // 128) for _ in range(B)]
        sl = lax.broadcasted_iota(jnp.int32, (8, 128), 0)
        for i in range(len(CUTS) - 1):
            with mark(f'wl{i}'):
                wait_cut(i)
            for r in range(CUTS[i], CUTS[i + 1], 8):
                a, row = divmod(VH[r // D] * D + r % D, 1024)
                w = wo_buf[a, row:row + 8].astype(F32)
                for b in range(B):
                    mul = mul_ref[b, r:r + 8, :]
                    for j in range(M // 128):
                        t = w[:, j * 128:(j + 1) * 128] * mul
                        part[b][j] = t if part[b][j] is None else part[b][j] + t

        def merge(lo, hi, k):
            m = (sl & k) != 0
            if k == 4:
                return jnp.where(m, hi, lo) + pltpu.roll(jnp.where(m, lo, hi), 4, 0)
            return jnp.where(m, hi, lo) + jnp.where(m, pltpu.roll(hi, k, 0), pltpu.roll(lo, 8 - k, 0))

        r4 = [[merge(part[b][j], part[b][j + 2], 4) for j in range(2)] for b in range(B)]
        r2 = [merge(r4[b][0], r4[b][1], 2) for b in range(B)]
        o_buf[...] = (base8 + g8 * merge(r2[0], r2[1], 1)).astype(BF16)
        o_copy.start()
        o_copy.wait()

    def kernel(*refs):
        if not REP:
            return body(*refs)

        def one(i):
            z = (i + 12345) * 1103515245; z = (z ^ (z >> 13)) * 1664525; z = z ^ (z >> 15)
            pl.delay(300 + (((z & 0xFFFF) * 3900) >> 16))
            with jax.named_scope('@x'):
                body(*refs)
        _loop(0, REP, one)

    def fn(A_x, A_c_kv, A_w_q, A_w_uk, A_w_uv, A_w_o, B_x, B_w1, B_b1, B_w2, B_b2):
        hbm = pl.BlockSpec(memory_space=pltpu.HBM)
        dma_sems = pltpu.SemaphoreType.DMA
        w1 = B_w1.reshape(M // 8, 8, F // 128, 128).transpose(0, 2, 1, 3).reshape(112, 64, 128)
        out = pl.pallas_call(
            kernel,
            out_shape=jax.ShapeDtypeStruct((8, 128), BF16),
            in_specs=[hbm] * 10,
            out_specs=hbm,
            scratch_shapes=[
                pltpu.VMEM((B, M), BF16), pltpu.VMEM((F,), BF16), pltpu.VMEM((M,), BF16),
                pltpu.VMEM((2048, 16, DC), BF16), pltpu.VMEM(W_VIEW, BF16), pltpu.VMEM(W_VIEW, BF16),
                pltpu.VMEM(W_VIEW, BF16), pltpu.VMEM(O_VIEW, BF16),
                pltpu.VMEM((112, 64, 128), BF16), pltpu.VMEM((112, 16, M), BF16),
                pltpu.VMEM((B, M, 128), F32),
                pltpu.VMEM((DC * 8 + 8, 128), F32),
                pltpu.VMEM((B * H, DC), BF16), pltpu.VMEM((B * H, DC), F32),
                pltpu.VMEM((B * H, 128), F32), pltpu.VMEM((B * H, 128), F32),
                pltpu.VMEM((H // HG, DC // 128, B, HG, 128 * HG), BF16), pltpu.VMEM((128, 128 * HG), BF16),
                pltpu.VMEM((3 * H, D), F32), pltpu.VMEM((B, 4 * D, 128), F32), pltpu.VMEM((8, 128), BF16),
                dma_sems((5,)), dma_sems((16,)), dma_sems((len(GROUPS) + len(CUTS) - 2,)), dma_sems((3,)),
            ],
            compiler_params=pltpu.CompilerParams(
                vmem_limit_bytes=100 * 1024 * 1024, disable_semaphore_checks=True, disable_bounds_checks=True, flags=FLAGS),
        )(A_x.reshape(B, M), A_c_kv.reshape(C_VIEW), A_w_q.reshape(W_VIEW), A_w_uk.reshape(W_VIEW),
          A_w_uv.reshape(W_VIEW), A_w_o.reshape(O_VIEW), w1, B_b1, B_w2.reshape(112, 16, M), B_b2)
        return out.reshape(M // 128, B, 128).transpose(1, 0, 2).reshape(B, 1, M)
    return fn


_impl = make(CTH=(1,1,0))


@jax.jit
def pallas_recurrent_scan__compressed_kv_cla__dense_activation_gelu__decode_kernel(
    A_x, A_c_kv, A_w_q, A_w_uk, A_w_uv, A_w_o, B_x, B_w1, B_b1, B_w2, B_b2,
):
    return _impl(A_x, A_c_kv, A_w_q, A_w_uk, A_w_uv, A_w_o, B_x, B_w1, B_b1, B_w2, B_b2)
```

```python
import contextlib
import jax
import jax.numpy as jnp
from jax import lax
import jax.experimental.pallas as pl
import jax.experimental.pallas.tpu as pltpu

F32 = jnp.float32
BF16 = jnp.bfloat16
B, H, SK, D, M, DC, F = 2, 32, 16384, 128, 512, 512, 1792
LOG2E = 1.4426950408889634
NT = (((1,), (1,)), ((), ()))
W_VIEW = (4, 128, H, D)
O_VIEW = (4, 8 * D, M)
HG = 16


def _loop(lo, hi, body):
    lax.fori_loop(lo, hi, lambda i, _: body(i), None)


def _rows8(v):
    return jnp.concatenate([v[:, j * 128:(j + 1) * 128] for j in range(M // 128)], axis=0)


def make(LEAD=26, IL=26, MERGE=True, SPLIT=7, CUTS=(0, 128, 256, 320, 384, 432, 464, 496, 512), PH1=48, PH2=33, PERM=True, TA='0110110110110111', TB='0101', TC='01010101', DMA_ONLY=False, REP=0, TR=False,
         CI=(0, 60, 100), CTH=(0, 1, 1, 1), HEAD=(0, 8, 16, 24), IG=(0, 1, 1), FLAGS=None, MG=((0, 1), (2,)), HG=16):
    mark = (lambda n: jax.named_scope('@' + n)) if TR else (lambda n: contextlib.nullcontext())
    C_VIEW = (4, 8192, DC) if PERM else (32, 1024, DC)
    E8 = (0, 2, 4, 6, 1, 3, 5, 7)
    VH = tuple(4 * a + 3 for a in E8)
    GROUPS = (0, 8, 16, 24, 30, 32)
    NG = len(GROUPS) - 1
    order = [(j, h) for j in [30, 31] + list(range(IL)) for h in range(2)]
    order += [(k + j, h) for k in range(IL, 26, 4) for h in range(2) for j in range(4)]
    o_list = []
    for j, h in order:
        g = max(i for i, c in enumerate(GROUPS) if c <= j)
        o_list += [(0, 1, h * 512 + j * 16, 16, 0, M, 0, g), (1, 3, h * 512 + j * 16, 16, 0, M, 1, g)]
    cut = lambda r: NG + max(k for k, c in enumerate(CUTS) if c <= r)
    for i in range(32):
        a, row = divmod(VH[i // 4] * D + 32 + i % 4 * 16, 1024)
        if i < 32 - SPLIT:
            d = (a, 1, row, 16, 0, M, CTH[i % len(CTH)], cut(i * 16))
            p = o_list[-1]
            if MERGE and (p[0], p[1], p[2] + p[3], p[6:]) == (a, 1, row, d[6:]):
                o_list[-1] = p[:3] + (p[3] + 16,) + p[4:]
            else:
                o_list.append(d)
        else:
            o_list += [(a, 1, row + r, 8, c, 256, 1, cut(i * 16 + r)) for r in (0, 8) for c in (0, 256)]
    o_t1 = [d for d in o_list if d[6] == 1]
    o_prog, k = [], LEAD
    for d in o_list:
        if d[6] == 0:
            o_prog.append(d)
        elif k < len(o_t1):
            o_prog.append(o_t1[k]); k += 1

    def body(x_hbm, ckv_hbm, wq_hbm, wuk_hbm, wuv_hbm, wo_hbm, w1_hbm, b1_hbm, w2_hbm, b2_hbm, o_hbm,
             x_buf, b1_buf, b2_buf, c_buf, wq_buf, wuk_buf, wuv_buf, wo_buf, w1_buf, w2_buf,
             xs, t8, qa_ref, acc_ref, m_ref, l_ref, a_buf, e_buf, ctx_ref, mul_ref, g_ref, s_ref, o_buf,
             sems):
        def fetch(src, dst, sem, queue):
            pltpu.make_async_copy(src, dst, sem).start(priority=queue)

        def wait_filled(buf, sem):
            pltpu.make_async_copy(buf, buf, sem).wait()

        def when(c, f):
            if isinstance(c, bool):
                c and f()
            else:
                pl.when(c)(f)

        def w_run(i, a, n=1):
            hbm, buf = ((wq_hbm, wq_buf), (wuk_hbm, wuk_buf), (wuv_hbm, wuv_buf))[i]

            def f(j, q):
                idx = (pl.ds(a, n), pl.ds(j * 2, 2))
                fetch(hbm.at[idx], buf.at[idx], sems.at[i], q)
            return f

        def c_run(a, n=1):
            def f(j, q):
                row = j * 16 + (a % 8 * 1024 if PERM else 0)
                idx = (pl.ds(a // 8 if PERM else a, n), pl.ds(row if isinstance(j, int) else pl.multiple_of(row, 16), 16))
                fetch(ckv_hbm.at[idx], c_buf.at[idx], sems.at[8 + (j >> 3) + (8 if a >= 19 else 0)], q)
            return f

        def f_run(i, first, always=False):
            hbm, buf = ((w1_hbm, w1_buf), (w2_hbm, w2_buf))[i]

            def f(j, q):
                p = j + first
                go = lambda: fetch(hbm.at[p], buf.at[p], sems.at[3 + i], q)
                go() if always else when(p >= 0 if first < 0 else p < 112, go)
            return f

        def both(f, g):
            return lambda j, q: f(j, q) or g(j, q)

        fa, fb, fc = f_run(1, PH2 - 64), f_run(1, PH2, True), both(f_run(1, PH2 + 64), f_run(0, PH1 - 64))
        if PERM:
            pa = [f_run(0, PH1, True)] + [w_run(2 - i // 4, i % 4) for i in range(12)] + [c_run(a) for a in range(3)]
            ph_a = [(int(t), pa[i + k]) for t, (i, k) in zip(TA, [(i, k) for i in (0, 2, 4, 6, 1, 3, 5, 7) for k in (0, 8)])]
            ph_b = [(1, c_run(19, 2)), (int(TB[0]), c_run(21, 2)), (1, c_run(23, 2)), (int(TB[1]), c_run(25)), (int(TB[2]), fb),
                    (1, c_run(20, 2)), (1, c_run(22, 2)), (int(TB[3]), c_run(24)), (0, fa), (1, c_run(26)), (0, fc)]
            ph_c = [(int(t), c_run(3 + i, 2)) for t, i in zip(TC, (0, 2, 4, 6, 1, 3, 5, 7))]
        else:
            ph_a = [(0, f_run(0, PH1, True)), (1, w_run(2, 0, 3)), (0, w_run(2, 3)), (1, w_run(1, 0, 3)), (0, w_run(1, 3)),
                    (1, w_run(0, 0, 3)), (0, w_run(0, 3)), (1, c_run(0, 3))]
            ph_b = [d for a in (19, 23, 27) for d in ((0, c_run(a)), (1, c_run(a + 1, 3)))] + [(0, c_run(31)), (0, fa), (1, fb), (0, fc)]
            ph_c = [d for a in (3, 7, 11, 15) for d in ((0, c_run(a)), (1, c_run(a + 1, 3)))]
        phases = (ph_a, ph_c, ph_b)
        ones = [[f for t, f in p if t] for p in phases]

        def desc_o(d):
            a, n, row, nr, col, nc, q, s = d
            idx = (pl.ds(a, n), pl.ds(row, nr), pl.ds(col, nc))
            fetch(wo_hbm.at[idx], wo_buf.at[idx], sems.at[24 + s], q)

        def program(v, j):
            out, k, n = [], LEAD, len(ones[v])
            for t, f in phases[v]:
                if not t:
                    out.append((0, lambda f=f: f(j, 0)))
                    continue
                if not isinstance(j, int) or j + k // n < 64:
                    out.append((1, lambda k=k: ones[v][k % n](j + k // n, 1)))
                elif v < 2:
                    r, i = divmod((j - 64) * n + k, len(ones[v + 1]))
                    out.append((1, lambda r=r, i=i: ones[v + 1][i](r, 1)))
                else:
                    out.append((1, lambda k=k: desc_o(o_t1[(j - 64) * n + k])))
                k += 1
            return out

        last = [64 - -(-LEAD // len(o)) for o in ones]

        def issue_rounds(v, lo, hi):
            _loop(lo, hi, lambda j: [f() for t, f in program(v, j)] and None)

        def issue_rest(v):
            for j in range(last[v], 64):
                for t, f in program(v, j):
                    f()

        def issue_o(k):
            with mark(f'io{k}'):
                for d in o_prog[CI[k]:(CI + (None,))[k + 1]]:
                    desc_o(d)

        x_copy = pltpu.make_async_copy(x_hbm, x_buf, sems.at[5 + 0])
        b1_copy = pltpu.make_async_copy(b1_hbm, b1_buf, sems.at[5 + 1])
        b2_copy = pltpu.make_async_copy(b2_hbm, b2_buf, sems.at[5 + 2])
        o_copy = pltpu.make_async_copy(o_buf, o_hbm, sems.at[5 + 0])
        first = program(0, 0) + program(0, 1)
        for g in range(LEAD):
            ones[0][g % len(ones[0])](g // len(ones[0]), 1)
            if g in HEAD:
                first.pop([t for t, f in first].index(0))[1]()
        for t, f in first:
            f()
        for c in (x_copy, b1_copy, b2_copy):
            c.start()

        def wait_keys(i):
            when(i < 8, lambda: wait_filled(c_buf.at[:, pl.ds(0, 19 * 128 // C_VIEW[0])], sems.at[8 + i]))
            when(i >= 8, lambda: wait_filled(c_buf.at[:, pl.ds(0, 13 * 128 // C_VIEW[0])], sems.at[8 + i]))

        def keys(a0, a1, g):
            if not PERM:
                return c_buf[pl.ds(a0, a1), pl.ds(pl.multiple_of(g * 128, 128), 128)].reshape(a1 * 128, DC)
            return jnp.concatenate([c_buf[(a0 + a) >> 3, pl.ds(pl.multiple_of(((a0 + a) & 7) * 1024 + g * 128, 128), 128)]
                                    for a in range(a1)], axis=0)

        def wait_group(g):
            lo, hi = GROUPS[g], GROUPS[g + 1]
            n = sum(d[1] * d[3] for d in o_list if d[7] == g)
            wait_filled(wo_buf.at[0, pl.ds(0, n)], sems.at[24 + g])

        def wait_cut(i):
            wait_filled(wo_buf.at[0, pl.ds(0, CUTS[i + 1] - CUTS[i])], sems.at[24 + NG + i])

        if DMA_ONLY:
            for v in range(3):
                issue_rounds(v, 0 if v else 2, last[v])
                issue_rest(v)
            for c in (x_copy, b1_copy, b2_copy):
                c.wait()
            for i, v in enumerate((wq_buf, wuk_buf, wuv_buf, w1_buf, w2_buf)):
                wait_filled(v, sems.at[i])
            for k in range(len(CI)):
                issue_o(k)
            for i in range(16):
                wait_keys(i)
            for g in range(len(GROUPS) - 1):
                wait_group(g)
            for i in range(len(CUTS) - 1):
                wait_cut(i)
            o_copy.start()
            o_copy.wait()
            return

        with mark('iA0'):
            issue_rounds(0, 2, 16)
        x_copy.wait()
        x = x_buf[...].astype(F32)
        xc = x - jnp.mean(x, axis=-1, keepdims=True)
        var = jnp.mean(xc * xc, axis=-1, keepdims=True)
        xn = (xc * lax.rsqrt(var + 1e-5)).astype(BF16)
        xf = xn.astype(F32)
        for b in range(B):
            for j in range(M // 128):
                cols = slice(j * 128, (j + 1) * 128)
                xs[b, cols, :] = jnp.broadcast_to(xf[b:b + 1, cols], (128, 128)).T
        e_buf[...] = (lax.broadcasted_iota(jnp.int32, (128, 128 * HG), 1) // HG
                      == lax.broadcasted_iota(jnp.int32, (128, 128 * HG), 0)).astype(F32).astype(BF16)
        m_ref[...] = jnp.full((B * H, 128), -jnp.inf, F32)
        l_ref[...] = jnp.zeros((B * H, 128), F32)
        acc_ref[...] = jnp.zeros((B * H, DC), F32)
        with mark('iA1'):
            issue_rounds(0, 16, last[0])
            issue_rest(0)
            issue_rounds(1, 0, 8)

        with mark('wq'):
            wait_filled(wq_buf, sems.at[0])

        def q_run(a, carry):
            def q_body(i, carry):
                q0, q1 = carry
                for u in range(8):
                    m = pl.ds(a * 128 + i * 8 + u, 1)
                    w = wq_buf[a, i * 8 + u].astype(F32)
                    q0 = q0 + xs[0, m, :] * w
                    q1 = q1 + xs[1, m, :] * w
                return q0, q1
            carry = lax.fori_loop(0, 16, q_body, carry)
            with mark('iq'):
                issue_rounds(1, 8 + 2 * a, 10 + 2 * a)
            return carry

        q0, q1 = lax.fori_loop(0, 4, q_run, (jnp.zeros((H, D), F32), jnp.zeros((H, D), F32)))
        q = jnp.concatenate([q0, q1, jnp.zeros((128 - B * H, D), F32)], axis=0).astype(BF16)

        wait_filled(wuk_buf, sems.at[1])
        group = (lax.broadcasted_iota(jnp.int32, (16, 8, 128), 2) % H) // 8

        def qa_body(i):
            for u in range(8):
                w = wuk_buf[i, pl.ds(u * 16, 16)].reshape(16 * H, D)
                r = lax.dot_general(w, q, NT, preferred_element_type=F32).reshape(16, 4, 8, 128)
                v = jnp.where(group == 0, r[:, 0],
                              jnp.where(group == 1, r[:, 1], jnp.where(group == 2, r[:, 2], r[:, 3])))
                t8[pl.ds(pl.multiple_of((i * 8 + u) * 128, 128), 128), :] = v.reshape(128, 128)
            with mark('iqa'):
                issue_rounds(1, 16 + 3 * i, 19 + 3 * i)

        _loop(0, 4, qa_body)
        sub = lax.broadcasted_iota(jnp.int32, (128, 128), 1) % 8
        for j in range(DC // 128):
            t = t8[pl.ds(j * 1024, 128, stride=8), :]
            for s in range(1, 8):
                t = jnp.where(sub == s, t8[pl.ds(j * 1024 + s, 128, stride=8), :], t)
            qa_ref[:, j * 128:(j + 1) * 128] = (t.T[:B * H] * (D ** -0.5 * LOG2E)).astype(BF16)

        wait_filled(wuv_buf, sems.at[2])
        b1_copy.wait()
        b2_copy.wait()
        x8 = _rows8(x)

        def gate():
            wait_filled(w1_buf, sems.at[3])
            wait_filled(w2_buf, sems.at[4])
            w1 = w1_buf[...].reshape(M // 8, F // 128, 8, 128)
            hid = jnp.concatenate([jnp.dot(xn, w1[:, n].reshape(M, 128), preferred_element_type=F32)
                                   for n in range(F // 128)], axis=1)
            hid = jax.nn.gelu(hid + b1_buf[...].astype(F32).reshape(1, F), approximate=True).astype(BF16)
            z = jnp.dot(hid, w2_buf[...].reshape(F, M), preferred_element_type=F32)
            z8 = _rows8(z + b2_buf[...].astype(F32).reshape(1, M))
            g_ref[...] = z8 * jax.nn.sigmoid(z8)

        def issue_c(lo, hi):
            with mark('ib'):
                for v in range(2):
                    issue_rounds(v + 1, jnp.maximum(lo - 64 * v, 0), jnp.minimum(hi - 64 * v, last[v + 1]))
                    pl.when(jnp.logical_and(lo < 64 * v + 62, hi >= 64 * v + 62))(lambda: issue_rest(v + 1))

        diag = (lax.broadcasted_iota(jnp.int32, (H, 128 * HG), 1) % HG
                == lax.broadcasted_iota(jnp.int32, (H, 128 * HG), 0) % HG)

        def block(i):
            upto = lambda k: jnp.maximum(30 + 6 * k, 8 * k + 14)
            issue_c(jnp.maximum(upto(i - 1) + 3, 28), upto(i))
            pl.when(i == 15)(lambda: issue_o(0))
            with mark('wc'):
                wait_keys(i)
            b = i >> 3
            hrows = pl.ds(pl.multiple_of(b * H, H), H)
            sc = lax.dot_general(qa_ref[hrows, :], keys(16 * b, 16, i & 7), NT, preferred_element_type=F32)
            m_prev = m_ref[hrows, :]
            m_new = jnp.maximum(m_prev, jnp.max(sc, axis=1, keepdims=True))
            p = jnp.exp2(sc - m_new[:, :1])
            alpha = jnp.exp2(m_prev - m_new)
            l_ref[hrows, :] = alpha * l_ref[hrows, :] + jnp.sum(p, axis=1, keepdims=True)
            m_ref[hrows, :] = m_new
            p = p.astype(BF16)
            issue_c(upto(i), upto(i) + 3)
            pv = jnp.dot(p, keys(16 * b, 16, i & 7), preferred_element_type=F32)
            acc_ref[hrows, :] = acc_ref[hrows, :] * alpha[:, :1] + pv

            @pl.when((i & 7) == 7)
            def _():
                pl.when(i == 15)(lambda: issue_o(1))
                pc = (acc_ref[hrows, :] / l_ref[hrows, :][:, :1]).astype(BF16)
                pc = jnp.concatenate([pc[:, j * 128:(j + 1) * 128] for j in range(DC // 128)], axis=0)
                rep = jnp.dot(pc, e_buf[...], preferred_element_type=F32)
                for j in range(DC // 128):
                    a = jnp.where(diag, rep[j * H:(j + 1) * H], 0.0).astype(BF16)
                    for hg in range(H // HG):
                        a_buf[hg, j, b] = a[hg * HG:(hg + 1) * HG]

            @pl.when(i == 15)
            def _():
                for hg in range(H // HG):
                    ctx = jnp.zeros((B * HG, D), F32)
                    for j in range(DC // 128):
                        ctx = ctx + jnp.dot(a_buf[hg, j].reshape(B * HG, 128 * HG),
                                            wuv_buf[j, :, hg * HG:(hg + 1) * HG].reshape(128 * HG, D),
                                            preferred_element_type=F32)
                    for b in range(B):
                        ctx_ref[b * H + hg * HG:b * H + (hg + 1) * HG] = ctx[b * HG:(b + 1) * HG]

        _loop(0, 16, block)
        issue_o(2)
        gate()
        for b in range(B):
            for i, h in enumerate(VH):
                cb = ctx_ref[b * H + h:b * H + h + 1].astype(BF16).astype(F32)
                mul_ref[b, i * D:(i + 1) * D] = jnp.broadcast_to(cb, (128, 128)).T
        g8 = g_ref[...]
        s_ref[...] = x8
        part = [[None] * (M // 128) for _ in range(B)]

        def vpu(i, lo, hi):
            for r in range(lo, hi, 8):
                a, row = divmod(VH[i] * D + r, 1024)
                w = wo_buf[a, row:row + 8].astype(F32)
                for b in range(B):
                    mul = mul_ref[b, i * D + r:i * D + r + 8, :]
                    for j in range(M // 128):
                        t = w[:, j * 128:(j + 1) * 128] * mul
                        part[b][j] = t if part[b][j] is None else part[b][j] + t

        wait_group(4)
        for gs in MG:
            with mark(f'wo{gs[0]}'):
                for g in gs:
                    wait_group(g)
            hs = [h for g in gs for h in range(g, H, 4) if h not in VH]
            lhs = [ctx_ref[pl.ds(h, B, stride=H), :] for h in hs]
            rhs = [wo_buf[h // 8, h % 8 * D:(h % 8 + 1) * D] for h in hs]
            s = jnp.dot(jnp.concatenate(lhs, axis=1).astype(BF16), jnp.concatenate(rhs, axis=0),
                        preferred_element_type=F32)
            s_ref[...] += _rows8(s) * g8
            if gs == MG[0]:
                for i in range(8):
                    vpu(i, 96, 128)
            if g == IG[2] - 1 and not IG[1]:
                issue_o(3)
        base8 = s_ref[...]

        with mark('wo3'):
            wait_group(3)
        for i in range(8):
            vpu(i, 0, 32)
        sl = lax.broadcasted_iota(jnp.int32, (8, 128), 0)
        for i in range(len(CUTS) - 1):
            with mark(f'wl{i}'):
                wait_cut(i)
            for r in range(CUTS[i], CUTS[i + 1], 8):
                vpu(r // 64, 32 + r % 64, 40 + r % 64)

        def merge(lo, hi, k):
            m = (sl & k) != 0
            if k == 4:
                return jnp.where(m, hi, lo) + pltpu.roll(jnp.where(m, lo, hi), 4, 0)
            return jnp.where(m, hi, lo) + jnp.where(m, pltpu.roll(hi, k, 0), pltpu.roll(lo, 8 - k, 0))

        r4 = [[merge(part[b][j], part[b][j + 2], 4) for j in range(2)] for b in range(B)]
        r2 = [merge(r4[b][0], r4[b][1], 2) for b in range(B)]
        o_buf[...] = (base8 + g8 * merge(r2[0], r2[1], 1)).astype(BF16)
        o_copy.start()
        o_copy.wait()

    def kernel(*refs):
        if not REP:
            return body(*refs)

        def one(i):
            z = (i + 12345) * 1103515245; z = (z ^ (z >> 13)) * 1664525; z = z ^ (z >> 15)
            pl.delay(300 + (((z & 0xFFFF) * 3900) >> 16))
            with jax.named_scope('@x'):
                body(*refs)
        _loop(0, REP, one)

    def fn(A_x, A_c_kv, A_w_q, A_w_uk, A_w_uv, A_w_o, B_x, B_w1, B_b1, B_w2, B_b2):
        hbm = pl.BlockSpec(memory_space=pltpu.HBM)
        dma_sems = pltpu.SemaphoreType.DMA
        w1 = B_w1.reshape(M // 8, 8, F // 128, 128).transpose(0, 2, 1, 3).reshape(112, 64, 128)
        out = pl.pallas_call(
            kernel,
            out_shape=jax.ShapeDtypeStruct((8, 128), BF16),
            in_specs=[hbm] * 10,
            out_specs=hbm,
            scratch_shapes=[
                pltpu.VMEM((B, M), BF16), pltpu.VMEM((F,), BF16), pltpu.VMEM((M,), BF16),
                pltpu.VMEM(C_VIEW, BF16), pltpu.VMEM(W_VIEW, BF16), pltpu.VMEM(W_VIEW, BF16),
                pltpu.VMEM(W_VIEW, BF16), pltpu.VMEM(O_VIEW, BF16),
                pltpu.VMEM((112, 64, 128), BF16), pltpu.VMEM((112, 16, M), BF16),
                pltpu.VMEM((B, M, 128), F32),
                pltpu.VMEM((DC * 8 + 8, 128), F32),
                pltpu.VMEM((B * H, DC), BF16), pltpu.VMEM((B * H, DC), F32),
                pltpu.VMEM((B * H, 128), F32), pltpu.VMEM((B * H, 128), F32),
                pltpu.VMEM((H // HG, DC // 128, B, HG, 128 * HG), BF16), pltpu.VMEM((128, 128 * HG), BF16),
                pltpu.VMEM((3 * H, D), F32), pltpu.VMEM((B, 8 * D, 128), F32), pltpu.VMEM((8, 128), F32), pltpu.VMEM((8, 128), F32), pltpu.VMEM((8, 128), BF16),
                dma_sems((22 + len(GROUPS) + len(CUTS),)),
            ],
            compiler_params=pltpu.CompilerParams(
                vmem_limit_bytes=100 * 1024 * 1024, disable_semaphore_checks=True, disable_bounds_checks=True, flags=FLAGS),
        )(A_x.reshape(B, M), A_c_kv.reshape(C_VIEW), A_w_q.reshape(W_VIEW), A_w_uk.reshape(W_VIEW),
          A_w_uv.reshape(W_VIEW), A_w_o.reshape(O_VIEW), w1, B_b1, B_w2.reshape(112, 16, M), B_b2)
        return out.reshape(M // 128, B, 128).transpose(1, 0, 2).reshape(B, 1, M)
    return fn


_impl = make()


@jax.jit
def pallas_recurrent_scan__compressed_kv_cla__dense_activation_gelu__decode_kernel(
    A_x, A_c_kv, A_w_q, A_w_uk, A_w_uv, A_w_o, B_x, B_w1, B_b1, B_w2, B_b2,
):
    return _impl(A_x, A_c_kv, A_w_q, A_w_uk, A_w_uv, A_w_o, B_x, B_w1, B_b1, B_w2, B_b2)
```

```python
import functools

import jax
import jax.numpy as jnp
from jax import lax
import jax.experimental.pallas as pl
import jax.experimental.pallas.tpu as pltpu

F32 = jnp.float32
BF16 = jnp.bfloat16

B, H, SK, D, M, DC, F = 2, 32, 16384, 128, 512, 512, 1792
LOG2E = 1.4426950408889634
NT = (((1,), (1,)), ((), ()))
HG = 16

LEAD = 26
W_VIEW = (4, 128, H, D)
C_VIEW = (4, 8 * 1024, DC)
C_BUF = (8, 5, 8 * 128, DC)
O_VIEW = (4, 2, 4 * D, M)
F_PIECES = M * F * 2 // 16384
O_GROUPS = ((0, D), (D, D), (2 * D, D), (3 * D, 32), (3 * D + 96, 32))
O_LAST = ((0, 2, 0, 416, 64), (2, 2, 0, 416, 64), (0, 1, 1, 416, 64), (1, 1, 1, 416, 64),
          (2, 1, 1, 416, 32), (2, 1, 1, 448, 32),
          (3, 1, 1, 416, 16), (3, 1, 1, 432, 16), (3, 1, 1, 448, 16), (3, 1, 1, 464, 8), (3, 1, 1, 472, 8))
S_WQ, S_WUK, S_WUV, S_W1, S_W2, S_X, S_B1, S_B2, S_C0, S_C1 = range(10)
S_C2, S_C3, S_O = S_C1 + 8, S_C1 + 16, S_C1 + 24
S_LAST = S_O + len(O_GROUPS)


def _loop(lo, hi, body):
    lax.fori_loop(lo, hi, lambda i, _: body(i), None)


def _rows16(row):
    return pl.ds(row if isinstance(row, int) else pl.multiple_of(row, 16), 16)


def _rows8(v):
    return jnp.concatenate([v[:, j * 128:(j + 1) * 128] for j in range(M // 128)], axis=0)


def _kernel(x_hbm, ckv_hbm, wq_hbm, wuk_hbm, wuv_hbm, wo_hbm, w1_hbm, b1_hbm, w2_hbm, b2_hbm,
            o_hbm,
            x_buf, b1_buf, b2_buf, c_buf, wq_buf, wuk_buf, wuv_buf, wo_buf, w1_buf, w2_buf,
            xs, t8, qa_ref, acc_ref, m_ref, l_ref, a_buf, e_buf, ctx_ref, mul_ref, s_ref, o_buf, sems):
    def fetch(src, dst, sem, queue):
        pltpu.make_async_copy(src, dst, sems.at[sem]).start(priority=queue)

    def wait_filled(buf, sem):
        pltpu.make_async_copy(buf, buf, sems.at[sem]).wait()

    def w_run(hbm, buf, sem, a):
        return lambda j, queue: fetch(hbm.at[a, pl.ds(j * 2, 2)], buf.at[a, pl.ds(j * 2, 2)], sem, queue)

    def c_run(a, n, sem):
        def run(j, queue):
            fetch(ckv_hbm.at[pl.ds(a // 8, n), _rows16(a % 8 * 1024 + j * 16)],
                  c_buf.at[j >> 3, pl.ds((a + 5) // 8, n), _rows16((a + 5) % 8 * 128 + (j & 7) * 16)],
                  sem if sem == S_C0 else sem + (j >> 3), queue)
        return run

    def f_run(hbm, buf, sem, first):
        def run(j, queue):
            p = first + j
            exists = p >= 0 if first < 0 else first + 64 <= F_PIECES or p < F_PIECES
            pl.when(exists)(lambda: fetch(hbm.at[p], buf.at[p], sem, queue))
        return run

    w1_run = functools.partial(f_run, w1_hbm, w1_buf, S_W1)
    w2_run = functools.partial(f_run, w2_hbm, w2_buf, S_W2)
    first = ([w1_run(48)] + [w_run(wuv_hbm, wuv_buf, S_WUV, a) for a in range(4)]
             + [w_run(wuk_hbm, wuk_buf, S_WUK, a) for a in range(4)]
             + [w_run(wq_hbm, wq_buf, S_WQ, a) for a in range(4)] + [c_run(a, 1, S_C0) for a in range(3)])
    order = (0, 2, 4, 6, 1, 3, 5, 7)
    phases = (
        list(zip((0, 1, 0, 1, 1, 0, 1, 0, 1, 1, 0, 1, 0, 1, 1, 1), [first[i + k] for i in order for k in (0, 8)])),
        [(i // 2 % 2, c_run(3 + i, 2, S_C1)) for i in order],
        [(1, c_run(19, 2, S_C2)), (0, c_run(21, 2, S_C2)), (1, c_run(23, 2, S_C2)),
         (0, c_run(25, 1, S_C3)), (1, w2_run(33)), (1, c_run(20, 2, S_C2)), (1, c_run(22, 2, S_C2)),
         (1, c_run(24, 1, S_C3)), (0, w2_run(-31)), (1, c_run(26, 1, S_C3)), (0, w2_run(97)), (0, w1_run(-16))],
    )
    ones = [[run for queue, run in phase if queue] for phase in phases]

    def o_copy(queue, sem, mib, half, row, cols=pl.ds(0, M)):
        idx = (mib, half, row, cols)
        return queue, functools.partial(fetch, wo_hbm.at[idx], wo_buf.at[idx], sem, queue)

    o_list = [o_copy(queue, S_O + g, pl.ds(queue, 1 + 2 * queue), half, pl.ds(row, 16))
              for g in (4, 0, 1, 2, 3) for row in range(O_GROUPS[g][0], sum(O_GROUPS[g]), 16)
              for half in range(2) for queue in range(2)]
    for i, (a0, n, half, row, rows) in enumerate(O_LAST):
        for a in range(a0, a0 + n):
            if rows == 64:
                o_list += [o_copy(0, S_LAST + i, a, half, pl.ds(row, 16)),
                           o_copy(1, S_LAST + i, a, half, pl.ds(row + 16, 48))]
            else:
                o_list += [o_copy(1, S_LAST + i, a, half, pl.ds(r, 8), pl.ds(c, 256))
                           for r in range(row, row + rows, 8) for c in (0, 256)]
    o_ones = [start for queue, start in o_list if queue]
    ahead = iter(o_ones[LEAD:])
    o_starts = [start for start in (next(ahead, None) if queue else start for queue, start in o_list) if start]

    def starts(v, j):
        out, k, n = [], LEAD, len(ones[v])
        for queue, run in phases[v]:
            if not queue:
                out.append(functools.partial(run, j, 0))
            elif not isinstance(j, int) or j + k // n < 64:
                out.append(functools.partial(ones[v][k % n], j + k // n, 1))
            elif v < 2:
                r, i = divmod((j - 64) * n + k, len(ones[v + 1]))
                out.append(functools.partial(ones[v + 1][i], r, 1))
            else:
                out.append(o_ones[(j - 64) * n + k])
            k += queue
        return out

    def issue(batch):
        for start in batch:
            start()

    inner = [64 - pl.cdiv(LEAD, len(o)) for o in ones]

    def issue_rounds(v, lo, hi):
        _loop(lo, hi, lambda j: issue(starts(v, j)))

    def issue_rest(v):
        for j in range(inner[v], 64):
            issue(starts(v, j))

    round0 = list(zip(phases[0], starts(0, 0)))
    for g in range(LEAD):
        ones[0][g % len(ones[0])](g // len(ones[0]), 1)
        if g % 12 == 0:
            round0.pop([queue for (queue, _), _ in round0].index(0))[1]()
    issue([start for _, start in round0] + starts(0, 1))
    fetch(x_hbm, x_buf, S_X, 0)
    fetch(b1_hbm, b1_buf, S_B1, 0)
    fetch(b2_hbm, b2_buf, S_B2, 0)
    issue_rounds(0, 2, 16)

    wait_filled(x_buf, S_X)
    x = x_buf[...].astype(F32)
    xc = x - jnp.mean(x, axis=-1, keepdims=True)
    var = jnp.mean(xc * xc, axis=-1, keepdims=True)
    xn = (xc * lax.rsqrt(var + 1e-5)).astype(BF16)
    xf = xn.astype(F32)
    for b in range(B):
        for j in range(M // 128):
            cols = slice(j * 128, (j + 1) * 128)
            xs[b, cols, :] = jnp.broadcast_to(xf[b:b + 1, cols], (128, 128)).T
    e_buf[...] = (lax.broadcasted_iota(jnp.int32, (128, 128 * HG), 1) // HG
                  == lax.broadcasted_iota(jnp.int32, (128, 128 * HG), 0)).astype(F32).astype(BF16)
    m_ref[...] = jnp.full((B * H, 128), -jnp.inf, F32)
    l_ref[...] = jnp.zeros((B * H, 128), F32)
    acc_ref[...] = jnp.zeros((B * H, DC), F32)
    s_ref[...] = _rows8(x)
    issue_rounds(0, 16, inner[0])
    issue_rest(0)
    issue_rounds(1, 0, 8)

    wait_filled(wq_buf, S_WQ)

    def q_run(a, carry):
        def q_body(i, carry):
            q0, q1 = carry
            for u in range(8):
                m = pl.ds(a * 128 + i * 8 + u, 1)
                w = wq_buf[a, i * 8 + u].astype(F32)
                q0 = q0 + xs[0, m, :] * w
                q1 = q1 + xs[1, m, :] * w
            return q0, q1

        carry = lax.fori_loop(0, 16, q_body, carry)
        issue_rounds(1, 8 + 2 * a, 10 + 2 * a)
        return carry

    q0, q1 = lax.fori_loop(0, 4, q_run, (jnp.zeros((H, D), F32), jnp.zeros((H, D), F32)))
    q = jnp.concatenate([q0, q1, jnp.zeros((128 - B * H, D), F32)], axis=0).astype(BF16)

    wait_filled(wuk_buf, S_WUK)
    group = (lax.broadcasted_iota(jnp.int32, (16, 8, 128), 2) % H) // 8

    def qa_run(a):
        for u in range(8):
            w = wuk_buf[a, pl.ds(u * 16, 16)].reshape(16 * H, D)
            r = lax.dot_general(w, q, NT, preferred_element_type=F32).reshape(16, 4, 8, 128)
            v = jnp.where(group == 0, r[:, 0],
                          jnp.where(group == 1, r[:, 1], jnp.where(group == 2, r[:, 2], r[:, 3])))
            t8[pl.ds(pl.multiple_of((a * 8 + u) * 128, 128), 128), :] = v.reshape(128, 128)
        issue_rounds(1, 16 + 3 * a, 19 + 3 * a)

    _loop(0, 4, qa_run)
    sub = lax.broadcasted_iota(jnp.int32, (128, 128), 1) % 8
    for j in range(DC // 128):
        t = t8[pl.ds(j * 1024, 128, stride=8), :]
        for s in range(1, 8):
            t = jnp.where(sub == s, t8[pl.ds(j * 1024 + s, 128, stride=8), :], t)
        qa_ref[:, j * 128:(j + 1) * 128] = (t.T[:B * H] * (D ** -0.5 * LOG2E)).astype(BF16)

    wait_filled(c_buf.at[:, 0, pl.ds(640, 384)], S_C0)
    wait_filled(wuv_buf, S_WUV)
    diag = (lax.broadcasted_iota(jnp.int32, (H, 128 * HG), 1) % HG
            == lax.broadcasted_iota(jnp.int32, (H, 128 * HG), 0) % HG)

    def started(i):
        return jnp.maximum(30 + 6 * i, 14 + 8 * i)

    def block(i):
        lo, hi = jnp.where(i == 8, started(7) + 4, jnp.maximum(started(i - 1), 28)), started(i)
        for v, v0 in ((1, 0), (2, 64)):
            issue_rounds(v, jnp.maximum(lo - v0, 0), jnp.minimum(hi - v0, inner[v]))
            pl.when(jnp.logical_and(lo < v0 + 62, hi >= v0 + 62))(lambda: issue_rest(v))
        pl.when(i == 15)(lambda: issue(o_starts[:60]))

        b, g = i >> 3, i & 7
        pl.when(b == 0)(lambda: wait_filled(c_buf.at[g, pl.ds(1, 2)], S_C1 + g))
        pl.when(b == 1)(lambda: wait_filled(c_buf.at[g, pl.ds(3, 2), pl.ds(0, 640)], S_C2 + g))
        pl.when(b == 1)(lambda: wait_filled(c_buf.at[g, 3, pl.ds(640, 384)], S_C3 + g))
        c = jnp.concatenate([c_buf[g, 2 * b, 640:], c_buf[g, 2 * b + 1], c_buf[g, 2 * b + 2, :640]], axis=0)
        hrows = pl.ds(pl.multiple_of(b * H, H), H)
        sc = lax.dot_general(qa_ref[hrows, :], c, NT, preferred_element_type=F32)
        m_prev = m_ref[hrows, :]
        m_new = jnp.maximum(m_prev, jnp.max(sc, axis=1, keepdims=True))
        p = jnp.exp2(sc - m_new[:, :1])
        alpha = jnp.exp2(m_prev - m_new)
        l_ref[hrows, :] = alpha * l_ref[hrows, :] + jnp.sum(p, axis=1, keepdims=True)
        m_ref[hrows, :] = m_new
        pv = jnp.dot(p.astype(BF16), c, preferred_element_type=F32)
        acc_ref[hrows, :] = acc_ref[hrows, :] * alpha[:, :1] + pv

        @pl.when(g == 7)
        def _():
            pl.when(b == 0)(lambda: issue_rounds(2, hi - 64, hi - 60))
            pl.when(b == 1)(lambda: issue(o_starts[60:100]))
            pc = (acc_ref[hrows, :] / l_ref[hrows, :][:, :1]).astype(BF16)
            pc = jnp.concatenate([pc[:, j * 128:(j + 1) * 128] for j in range(DC // 128)], axis=0)
            rep = jnp.dot(pc, e_buf[...], preferred_element_type=F32)
            for j in range(DC // 128):
                a = jnp.where(diag, rep[j * H:(j + 1) * H], 0.0).astype(BF16)
                for k in range(H // HG):
                    a_buf[k, j, b] = a[k * HG:(k + 1) * HG]

        @pl.when(i == 15)
        def _():
            for k in range(H // HG):
                ctx = sum(jnp.dot(a_buf[k, j].reshape(B * HG, 128 * HG),
                                  wuv_buf[j, :, k * HG:(k + 1) * HG].reshape(128 * HG, D),
                                  preferred_element_type=F32) for j in range(DC // 128))
                for r in range(B):
                    ctx_ref[r * H + k * HG:r * H + (k + 1) * HG] = ctx[r * HG:(r + 1) * HG]

    _loop(0, 16, block)
    issue(o_starts[100:])

    wait_filled(w1_buf, S_W1)
    wait_filled(w2_buf, S_W2)
    wait_filled(b1_buf, S_B1)
    wait_filled(b2_buf, S_B2)
    w1 = w1_buf[...].reshape(M // 8, F // 128, 8, 128)
    hid = jnp.concatenate([jnp.dot(xn, w1[:, n].reshape(M, 128), preferred_element_type=F32)
                           for n in range(F // 128)], axis=1)
    hid = jax.nn.gelu(hid + b1_buf[...].astype(F32).reshape(1, F), approximate=True).astype(BF16)
    z = jnp.dot(hid, w2_buf[...].reshape(F, M), preferred_element_type=F32)
    z8 = _rows8(z + b2_buf[...].astype(F32).reshape(1, M))
    g8 = z8 * jax.nn.sigmoid(z8)

    for b in range(B):
        for a in range(H // 4):
            r = b * H + 4 * a + 3
            mul_ref[b, a] = jnp.broadcast_to(ctx_ref[r:r + 1].astype(BF16).astype(F32), (128, 128)).T

    def wait_group(g):
        wait_filled(wo_buf.at[:, :, pl.ds(*O_GROUPS[g])], S_O + g)

    def project(lo, hi):
        lhs = jnp.concatenate([ctx_ref[pl.ds(h, B, stride=H), :] for h in range(H) if lo <= h % 4 < hi], axis=1)
        rhs = wo_buf[:, :, lo * D:hi * D].reshape(8 * (hi - lo) * D, M)
        s_ref[...] += _rows8(jnp.dot(lhs.astype(BF16), rhs, preferred_element_type=F32)) * g8

    part = [[None] * (M // 128) for _ in range(B)]

    def accumulate(a0, n, half, row, rows):
        for a in range(a0, a0 + n):
            for r in range(row, row + rows, 8):
                w = wo_buf[a, half, r:r + 8].astype(F32)
                for b in range(B):
                    mul = mul_ref[b, 2 * a + half, r - 3 * D:r - 3 * D + 8]
                    for j in range(M // 128):
                        t = w[:, j * 128:(j + 1) * 128] * mul
                        part[b][j] = t if part[b][j] is None else part[b][j] + t

    for g in (4, 0, 1):
        wait_group(g)
    project(0, 2)
    for half in range(2):
        accumulate(0, 4, half, *O_GROUPS[4])
    wait_group(2)
    project(2, 3)
    base8 = s_ref[...]
    wait_group(3)
    for half in range(2):
        accumulate(0, 4, half, *O_GROUPS[3])
    for i, (a0, n, half, row, rows) in enumerate(O_LAST):
        wait_filled(wo_buf.at[pl.ds(a0, n), half, pl.ds(row, rows)], S_LAST + i)
        accumulate(a0, n, half, row, rows)

    sl = lax.broadcasted_iota(jnp.int32, (8, 128), 0)

    def merge(lo, hi, k):
        m = (sl & k) != 0
        if k == 4:
            return jnp.where(m, hi, lo) + pltpu.roll(jnp.where(m, lo, hi), 4, 0)
        return jnp.where(m, hi, lo) + jnp.where(m, pltpu.roll(hi, k, 0), pltpu.roll(lo, 8 - k, 0))

    r4 = [[merge(part[b][j], part[b][j + 2], 4) for j in range(2)] for b in range(B)]
    r2 = [merge(r4[b][0], r4[b][1], 2) for b in range(B)]
    o_buf[...] = (base8 + g8 * merge(r2[0], r2[1], 1)).astype(BF16)
    store = pltpu.make_async_copy(o_buf, o_hbm, sems.at[S_X])
    store.start()
    store.wait()


@jax.jit
def pallas_recurrent_scan__compressed_kv_cla__dense_activation_gelu__decode_kernel(
    A_x: jax.Array,
    A_c_kv: jax.Array,
    A_w_q: jax.Array,
    A_w_uk: jax.Array,
    A_w_uv: jax.Array,
    A_w_o: jax.Array,
    B_x: jax.Array,
    B_w1: jax.Array,
    B_b1: jax.Array,
    B_w2: jax.Array,
    B_b2: jax.Array,
):
    del B_x
    hbm = pl.BlockSpec(memory_space=pltpu.HBM)
    w1_view, w2_view = (F_PIECES, 64, 128), (F_PIECES, 16, M)
    w1 = B_w1.reshape(M // 8, 8, F // 128, 128).transpose(0, 2, 1, 3).reshape(w1_view)
    out = pl.pallas_call(
        _kernel,
        out_shape=jax.ShapeDtypeStruct((8, 128), BF16),
        in_specs=[hbm] * 10,
        out_specs=hbm,
        scratch_shapes=[
            pltpu.VMEM((B, M), BF16), pltpu.VMEM((F,), BF16), pltpu.VMEM((M,), BF16),
            pltpu.VMEM(C_BUF, BF16), pltpu.VMEM(W_VIEW, BF16), pltpu.VMEM(W_VIEW, BF16),
            pltpu.VMEM(W_VIEW, BF16), pltpu.VMEM(O_VIEW, BF16),
            pltpu.VMEM(w1_view, BF16), pltpu.VMEM(w2_view, BF16),
            pltpu.VMEM((B, M, 128), F32),
            pltpu.VMEM((DC * 8 + 8, 128), F32),
            pltpu.VMEM((B * H, DC), BF16), pltpu.VMEM((B * H, DC), F32),
            pltpu.VMEM((B * H, 128), F32), pltpu.VMEM((B * H, 128), F32),
            pltpu.VMEM((H // HG, DC // 128, B, HG, 128 * HG), BF16), pltpu.VMEM((128, 128 * HG), BF16),
            pltpu.VMEM((3 * H, D), F32), pltpu.VMEM((B, H // 4, D, 128), F32),
            pltpu.VMEM((8, 128), F32), pltpu.VMEM((8, 128), BF16),
            pltpu.SemaphoreType.DMA((S_LAST + len(O_LAST),)),
        ],
        compiler_params=pltpu.CompilerParams(
            vmem_limit_bytes=100 * 1024 * 1024, disable_semaphore_checks=True, disable_bounds_checks=True),
    )(A_x.reshape(B, M), A_c_kv.reshape(C_VIEW), A_w_q.reshape(W_VIEW), A_w_uk.reshape(W_VIEW),
      A_w_uv.reshape(W_VIEW), A_w_o.reshape(O_VIEW), w1, B_b1, B_w2.reshape(w2_view), B_b2)
    return out.reshape(M // 128, B, 128).transpose(1, 0, 2).reshape(B, 1, M)
```

```python
import functools

import jax
import jax.numpy as jnp
from jax import lax
import jax.experimental.pallas as pl
import jax.experimental.pallas.tpu as pltpu

F32 = jnp.float32
BF16 = jnp.bfloat16

B, H, SK, D, M, DC, F = 2, 32, 16384, 128, 512, 512, 1792
LOG2E = 1.4426950408889634
NT = (((1,), (1,)), ((), ()))
HG = 16

LEAD = 26
W_VIEW = (4, 128, H, D)
C_VIEW = (4, 8 * 1024, DC)
C_BUF = (8, 5, 8 * 128, DC)
O_VIEW = (4, 2, 4 * D, M)
F_PIECES = M * F * 2 // 16384
O_GROUPS = ((0, D), (D, D), (2 * D, D), (3 * D, 32), (3 * D + 96, 32))
O_LAST = ((0, 2, 0, 416, 64), (2, 2, 0, 416, 64), (0, 1, 1, 416, 64), (1, 1, 1, 416, 64),
          (2, 1, 1, 416, 32), (2, 1, 1, 448, 32),
          (3, 1, 1, 416, 16), (3, 1, 1, 432, 16), (3, 1, 1, 448, 16), (3, 1, 1, 464, 8), (3, 1, 1, 472, 8))
S_WQ, S_WUK, S_WUV, S_W1, S_W2, S_X, S_B1, S_B2, S_C0, S_C1 = range(10)
S_C2, S_C3, S_O = S_C1 + 8, S_C1 + 16, S_C1 + 24
S_LAST = S_O + len(O_GROUPS)


def _loop(lo, hi, body):
    lax.fori_loop(lo, hi, lambda i, _: body(i), None)


def _rows16(row):
    return pl.ds(row if isinstance(row, int) else pl.multiple_of(row, 16), 16)


def _rows8(v):
    return jnp.concatenate([v[:, j * 128:(j + 1) * 128] for j in range(M // 128)], axis=0)


def _kernel(x_hbm, ckv_hbm, wq_hbm, wuk_hbm, wuv_hbm, wo_hbm, w1_hbm, b1_hbm, w2_hbm, b2_hbm,
            o_hbm,
            x_buf, b1_buf, b2_buf, c_buf, wq_buf, wuk_buf, wuv_buf, wo_buf, w1_buf, w2_buf,
            xs, t8, qa_ref, acc_ref, m_ref, l_ref, a_buf, e_buf, ctx_ref, mul_ref, s_ref, o_buf, sems):
    def fetch(src, dst, sem, queue):
        pltpu.make_async_copy(src, dst, sems.at[sem]).start(priority=queue)

    def wait_filled(buf, sem):
        pltpu.make_async_copy(buf, buf, sems.at[sem]).wait()

    def w_run(hbm, buf, sem, a):
        return lambda j, queue: fetch(hbm.at[a, pl.ds(j * 2, 2)], buf.at[a, pl.ds(j * 2, 2)], sem, queue)

    def c_run(a, n, sem):
        def run(j, queue):
            fetch(ckv_hbm.at[pl.ds(a // 8, n), _rows16(a % 8 * 1024 + j * 16)],
                  c_buf.at[j >> 3, pl.ds((a + 5) // 8, n), _rows16((a + 5) % 8 * 128 + (j & 7) * 16)],
                  sem if sem == S_C0 else sem + (j >> 3), queue)
        return run

    def f_run(hbm, buf, sem, first):
        def run(j, queue):
            p = first + j
            exists = p >= 0 if first < 0 else first + 64 <= F_PIECES or p < F_PIECES
            pl.when(exists)(lambda: fetch(hbm.at[p], buf.at[p], sem, queue))
        return run

    w1_run = functools.partial(f_run, w1_hbm, w1_buf, S_W1)
    w2_run = functools.partial(f_run, w2_hbm, w2_buf, S_W2)
    first = ([w1_run(48)] + [w_run(wuv_hbm, wuv_buf, S_WUV, a) for a in range(4)]
             + [w_run(wuk_hbm, wuk_buf, S_WUK, a) for a in range(4)]
             + [w_run(wq_hbm, wq_buf, S_WQ, a) for a in range(4)] + [c_run(a, 1, S_C0) for a in range(3)])
    order = (0, 2, 4, 6, 1, 3, 5, 7)
    phases = (
        list(zip((0, 1, 0, 1, 1, 0, 1, 0, 1, 1, 0, 1, 0, 1, 1, 1), [first[i + k] for i in order for k in (0, 8)])),
        [(i // 2 % 2, c_run(3 + i, 2, S_C1)) for i in order],
        [(1, c_run(19, 2, S_C2)), (0, c_run(21, 2, S_C2)), (1, c_run(23, 2, S_C2)),
         (0, c_run(25, 1, S_C3)), (1, w2_run(33)), (0, c_run(20, 2, S_C2)), (1, c_run(22, 2, S_C2)),
         (1, c_run(24, 1, S_C3)), (0, w2_run(-31)), (1, c_run(26, 1, S_C3)), (0, w2_run(97)), (0, w1_run(-16))],
    )
    ones = [[run for queue, run in phase if queue] for phase in phases]

    def o_copy(queue, sem, mib, half, row, cols=pl.ds(0, M)):
        idx = (mib, half, row, cols)
        return queue, functools.partial(fetch, wo_hbm.at[idx], wo_buf.at[idx], sem, queue)

    o_list = [o_copy(queue, S_O + g, pl.ds(queue, 1 + 2 * queue), half, pl.ds(row, 16))
              for g in (4, 0, 1, 2, 3) for row in range(O_GROUPS[g][0], sum(O_GROUPS[g]), 16)
              for half in range(2) for queue in range(2)]
    for i, (a0, n, half, row, rows) in enumerate(O_LAST):
        for a in range(a0, a0 + n):
            if rows == 64:
                o_list += [o_copy(0, S_LAST + i, a, half, pl.ds(row, 16)),
                           o_copy(1, S_LAST + i, a, half, pl.ds(row + 16, 48))]
            else:
                o_list += [o_copy(1, S_LAST + i, a, half, pl.ds(r, 8), pl.ds(c, 256))
                           for r in range(row, row + rows, 8) for c in (0, 256)]
    o_ones = [start for queue, start in o_list if queue]
    ahead = iter(o_ones[LEAD:])
    o_starts = [start for start in (next(ahead, None) if queue else start for queue, start in o_list) if start]

    def starts(v, j):
        out, k, n = [], LEAD, len(ones[v])
        for queue, run in phases[v]:
            if not queue:
                out.append(functools.partial(run, j, 0))
            elif not isinstance(j, int) or j + k // n < 64:
                out.append(functools.partial(ones[v][k % n], j + k // n, 1))
            elif v < 2:
                r, i = divmod((j - 64) * n + k, len(ones[v + 1]))
                out.append(functools.partial(ones[v + 1][i], r, 1))
            else:
                out.append(o_ones[(j - 64) * n + k])
            k += queue
        return out

    def issue(batch):
        for start in batch:
            start()

    inner = [64 - pl.cdiv(LEAD, len(o)) for o in ones]

    def issue_rounds(v, lo, hi):
        _loop(lo, hi, lambda j: issue(starts(v, j)))

    def issue_rest(v):
        for j in range(inner[v], 64):
            issue(starts(v, j))

    round0 = list(zip(phases[0], starts(0, 0)))
    for g in range(LEAD):
        ones[0][g % len(ones[0])](g // len(ones[0]), 1)
        if g % 12 == 0:
            round0.pop([queue for (queue, _), _ in round0].index(0))[1]()
    issue([start for _, start in round0] + starts(0, 1))
    fetch(x_hbm, x_buf, S_X, 0)
    fetch(b1_hbm, b1_buf, S_B1, 0)
    fetch(b2_hbm, b2_buf, S_B2, 0)
    issue_rounds(0, 2, 16)

    wait_filled(x_buf, S_X)
    x = x_buf[...].astype(F32)
    xc = x - jnp.mean(x, axis=-1, keepdims=True)
    var = jnp.mean(xc * xc, axis=-1, keepdims=True)
    xn = (xc * lax.rsqrt(var + 1e-5)).astype(BF16)
    xf = xn.astype(F32)
    for b in range(B):
        for j in range(M // 128):
            cols = slice(j * 128, (j + 1) * 128)
            xs[b, cols, :] = jnp.broadcast_to(xf[b:b + 1, cols], (128, 128)).T
    e_buf[...] = (lax.broadcasted_iota(jnp.int32, (128, 128 * HG), 1) // HG
                  == lax.broadcasted_iota(jnp.int32, (128, 128 * HG), 0)).astype(F32).astype(BF16)
    m_ref[...] = jnp.full((B * H, 128), -jnp.inf, F32)
    l_ref[...] = jnp.zeros((B * H, 128), F32)
    acc_ref[...] = jnp.zeros((B * H, DC), F32)
    s_ref[...] = _rows8(x)
    issue_rounds(0, 16, inner[0])
    issue_rest(0)
    issue_rounds(1, 0, 8)

    wait_filled(wq_buf, S_WQ)

    def q_run(a, carry):
        def q_body(i, carry):
            q0, q1 = carry
            for u in range(8):
                m = pl.ds(a * 128 + i * 8 + u, 1)
                w = wq_buf[a, i * 8 + u].astype(F32)
                q0 = q0 + xs[0, m, :] * w
                q1 = q1 + xs[1, m, :] * w
            return q0, q1

        carry = lax.fori_loop(0, 16, q_body, carry)
        issue_rounds(1, 8 + 2 * a, 10 + 2 * a)
        return carry

    q0, q1 = lax.fori_loop(0, 4, q_run, (jnp.zeros((H, D), F32), jnp.zeros((H, D), F32)))
    q = jnp.concatenate([q0, q1, jnp.zeros((128 - B * H, D), F32)], axis=0).astype(BF16)

    wait_filled(wuk_buf, S_WUK)
    group = (lax.broadcasted_iota(jnp.int32, (16, 8, 128), 2) % H) // 8

    def qa_run(a):
        for u in range(8):
            w = wuk_buf[a, pl.ds(u * 16, 16)].reshape(16 * H, D)
            r = lax.dot_general(w, q, NT, preferred_element_type=F32).reshape(16, 4, 8, 128)
            v = jnp.where(group == 0, r[:, 0],
                          jnp.where(group == 1, r[:, 1], jnp.where(group == 2, r[:, 2], r[:, 3])))
            t8[pl.ds(pl.multiple_of((a * 8 + u) * 128, 128), 128), :] = v.reshape(128, 128)
        issue_rounds(1, 16 + 3 * a, 19 + 3 * a)

    _loop(0, 4, qa_run)
    sub = lax.broadcasted_iota(jnp.int32, (128, 128), 1) % 8
    for j in range(DC // 128):
        t = t8[pl.ds(j * 1024, 128, stride=8), :]
        for s in range(1, 8):
            t = jnp.where(sub == s, t8[pl.ds(j * 1024 + s, 128, stride=8), :], t)
        qa_ref[:, j * 128:(j + 1) * 128] = (t.T[:B * H] * (D ** -0.5 * LOG2E)).astype(BF16)

    wait_filled(c_buf.at[:, 0, pl.ds(640, 384)], S_C0)
    wait_filled(wuv_buf, S_WUV)
    diag = (lax.broadcasted_iota(jnp.int32, (H, 128 * HG), 1) % HG
            == lax.broadcasted_iota(jnp.int32, (H, 128 * HG), 0) % HG)

    def started(i):
        return jnp.maximum(30 + 6 * i, 15 + 8 * i)

    def block(i):
        lo, hi = jnp.where(i == 8, started(7) + 4, jnp.maximum(started(i - 1), 28)), started(i)
        for v, v0 in ((1, 0), (2, 64)):
            issue_rounds(v, jnp.maximum(lo - v0, 0), jnp.minimum(hi - v0, inner[v]))
            pl.when(jnp.logical_and(lo < v0 + 62, hi >= v0 + 62))(lambda: issue_rest(v))
        pl.when(i == 15)(lambda: issue(o_starts[:60]))

        b, g = i >> 3, i & 7
        pl.when(b == 0)(lambda: wait_filled(c_buf.at[g, pl.ds(1, 2)], S_C1 + g))
        pl.when(b == 1)(lambda: wait_filled(c_buf.at[g, pl.ds(3, 2), pl.ds(0, 640)], S_C2 + g))
        pl.when(b == 1)(lambda: wait_filled(c_buf.at[g, 3, pl.ds(640, 384)], S_C3 + g))
        c = jnp.concatenate([c_buf[g, 2 * b, 640:], c_buf[g, 2 * b + 1], c_buf[g, 2 * b + 2, :640]], axis=0)
        hrows = pl.ds(pl.multiple_of(b * H, H), H)
        sc = lax.dot_general(qa_ref[hrows, :], c, NT, preferred_element_type=F32)
        m_prev = m_ref[hrows, :]
        m_new = jnp.maximum(m_prev, jnp.max(sc, axis=1, keepdims=True))
        p = jnp.exp2(sc - m_new[:, :1])
        alpha = jnp.exp2(m_prev - m_new)
        l_ref[hrows, :] = alpha * l_ref[hrows, :] + jnp.sum(p, axis=1, keepdims=True)
        m_ref[hrows, :] = m_new
        pv = jnp.dot(p.astype(BF16), c, preferred_element_type=F32)
        acc_ref[hrows, :] = acc_ref[hrows, :] * alpha[:, :1] + pv

        @pl.when(g == 7)
        def _():
            pl.when(b == 0)(lambda: issue_rounds(2, hi - 64, hi - 60))
            pl.when(b == 1)(lambda: issue(o_starts[60:100]))
            pc = (acc_ref[hrows, :] / l_ref[hrows, :][:, :1]).astype(BF16)
            pc = jnp.concatenate([pc[:, j * 128:(j + 1) * 128] for j in range(DC // 128)], axis=0)
            rep = jnp.dot(pc, e_buf[...], preferred_element_type=F32)
            for j in range(DC // 128):
                a = jnp.where(diag, rep[j * H:(j + 1) * H], 0.0).astype(BF16)
                for k in range(H // HG):
                    a_buf[k, j, b] = a[k * HG:(k + 1) * HG]

        @pl.when(i == 15)
        def _():
            for k in range(H // HG):
                ctx = sum(jnp.dot(a_buf[k, j].reshape(B * HG, 128 * HG),
                                  wuv_buf[j, :, k * HG:(k + 1) * HG].reshape(128 * HG, D),
                                  preferred_element_type=F32) for j in range(DC // 128))
                for r in range(B):
                    ctx_ref[r * H + k * HG:r * H + (k + 1) * HG] = ctx[r * HG:(r + 1) * HG]

    _loop(0, 16, block)
    issue(o_starts[100:])

    wait_filled(w1_buf, S_W1)
    wait_filled(w2_buf, S_W2)
    wait_filled(b1_buf, S_B1)
    wait_filled(b2_buf, S_B2)
    w1 = w1_buf[...].reshape(M // 8, F // 128, 8, 128)
    hid = jnp.concatenate([jnp.dot(xn, w1[:, n].reshape(M, 128), preferred_element_type=F32)
                           for n in range(F // 128)], axis=1)
    hid = jax.nn.gelu(hid + b1_buf[...].astype(F32).reshape(1, F), approximate=True).astype(BF16)
    z = jnp.dot(hid, w2_buf[...].reshape(F, M), preferred_element_type=F32)
    z8 = _rows8(z + b2_buf[...].astype(F32).reshape(1, M))
    g8 = z8 * jax.nn.sigmoid(z8)

    odd = lax.broadcasted_iota(jnp.int32, (1, D), 1) % 2 == 1
    for a in range(H // 4):
        c0, c1 = (ctx_ref[pl.ds(b * H + 4 * a + 3, 1), :].astype(BF16).astype(F32) for b in range(B))
        mul_ref[0, a] = jnp.broadcast_to(jnp.where(odd, c1, c0), (128, D)).T
        mul_ref[1, a] = jnp.broadcast_to(jnp.where(odd, c0, c1), (128, D)).T

    def wait_group(g):
        wait_filled(wo_buf.at[:, :, pl.ds(*O_GROUPS[g])], S_O + g)

    def project(lo, hi):
        lhs = jnp.concatenate([ctx_ref[pl.ds(h, B, stride=H), :] for h in range(H) if lo <= h % 4 < hi], axis=1)
        rhs = wo_buf[:, :, lo * D:hi * D].reshape(8 * (hi - lo) * D, M)
        s_ref[...] += _rows8(jnp.dot(lhs.astype(BF16), rhs, preferred_element_type=F32)) * g8

    part = [[None] * (M // 128) for _ in range(2)]

    def accumulate(a0, n, half, row, rows):
        for a in range(a0, a0 + n):
            for r in range(row, row + rows, 8):
                w = wo_buf[a, half, r:r + 8].astype(F32)
                for e in range(2):
                    mul = mul_ref[e, 2 * a + half, r - 3 * D:r - 3 * D + 8]
                    for j in range(M // 128):
                        t = w[:, j * 128:(j + 1) * 128] * mul
                        part[e][j] = t if part[e][j] is None else part[e][j] + t

    for g in (4, 0, 1):
        wait_group(g)
    project(0, 2)
    for half in range(2):
        accumulate(0, 4, half, *O_GROUPS[4])
    wait_group(2)
    project(2, 3)
    base8 = s_ref[...]
    wait_group(3)
    for half in range(2):
        accumulate(0, 4, half, *O_GROUPS[3])
    for i, (a0, n, half, row, rows) in enumerate(O_LAST):
        wait_filled(wo_buf.at[pl.ds(a0, n), half, pl.ds(row, rows)], S_LAST + i)
        accumulate(a0, n, half, row, rows)

    sl = lax.broadcasted_iota(jnp.int32, (8, 128), 0)

    def merge(lo, hi, k):
        m = (sl & k) != 0
        return jnp.where(m, hi, lo), pltpu.roll(jnp.where(m, lo, hi), k, 0)

    r1 = [part[0][j] + pltpu.roll(part[1][j], 1, 0) for j in range(4)]
    r2 = [jnp.add(*merge(r1[j], r1[j + 1], 2)) for j in (0, 2)]
    near, far = merge(r2[0], r2[1], 4)
    o_buf[...] = (base8 + g8 * near + g8 * far).astype(BF16)
    store = pltpu.make_async_copy(o_buf, o_hbm, sems.at[S_X])
    store.start()
    store.wait()


@jax.jit
def pallas_recurrent_scan__compressed_kv_cla__dense_activation_gelu__decode_kernel(
    A_x: jax.Array,
    A_c_kv: jax.Array,
    A_w_q: jax.Array,
    A_w_uk: jax.Array,
    A_w_uv: jax.Array,
    A_w_o: jax.Array,
    B_x: jax.Array,
    B_w1: jax.Array,
    B_b1: jax.Array,
    B_w2: jax.Array,
    B_b2: jax.Array,
):
    del B_x
    hbm = pl.BlockSpec(memory_space=pltpu.HBM)
    w1_view, w2_view = (F_PIECES, 64, 128), (F_PIECES, 16, M)
    w1 = B_w1.reshape(M // 8, 8, F // 128, 128).transpose(0, 2, 1, 3).reshape(w1_view)
    out = pl.pallas_call(
        _kernel,
        out_shape=jax.ShapeDtypeStruct((8, 128), BF16),
        in_specs=[hbm] * 10,
        out_specs=hbm,
        scratch_shapes=[
            pltpu.VMEM((B, M), BF16), pltpu.VMEM((F,), BF16), pltpu.VMEM((M,), BF16),
            pltpu.VMEM(C_BUF, BF16), pltpu.VMEM(W_VIEW, BF16), pltpu.VMEM(W_VIEW, BF16),
            pltpu.VMEM(W_VIEW, BF16), pltpu.VMEM(O_VIEW, BF16),
            pltpu.VMEM(w1_view, BF16), pltpu.VMEM(w2_view, BF16),
            pltpu.VMEM((B, M, 128), F32),
            pltpu.VMEM((DC * 8 + 8, 128), F32),
            pltpu.VMEM((B * H, DC), BF16), pltpu.VMEM((B * H, DC), F32),
            pltpu.VMEM((B * H, 128), F32), pltpu.VMEM((B * H, 128), F32),
            pltpu.VMEM((H // HG, DC // 128, B, HG, 128 * HG), BF16), pltpu.VMEM((128, 128 * HG), BF16),
            pltpu.VMEM((3 * H, D), F32), pltpu.VMEM((B, H // 4, D, 128), F32),
            pltpu.VMEM((8, 128), F32), pltpu.VMEM((8, 128), BF16),
            pltpu.SemaphoreType.DMA((S_LAST + len(O_LAST),)),
        ],
        compiler_params=pltpu.CompilerParams(
            vmem_limit_bytes=100 * 1024 * 1024, disable_semaphore_checks=True, disable_bounds_checks=True),
    )(A_x.reshape(B, M), A_c_kv.reshape(C_VIEW), A_w_q.reshape(W_VIEW), A_w_uk.reshape(W_VIEW),
      A_w_uv.reshape(W_VIEW), A_w_o.reshape(O_VIEW), w1, B_b1, B_w2.reshape(w2_view), B_b2)
    return out.reshape(M // 128, B, 128).transpose(1, 0, 2).reshape(B, 1, M)
```

```python
import functools

import jax
import jax.numpy as jnp
from jax import lax
import jax.experimental.pallas as pl
import jax.experimental.pallas.tpu as pltpu

F32 = jnp.float32
BF16 = jnp.bfloat16

B, H, SK, D, M, DC, F = 2, 32, 16384, 128, 512, 512, 1792
LOG2E = 1.4426950408889634
NT = (((1,), (1,)), ((), ()))
HG = 16

LEAD = 26
W_VIEW = (4, 128, H, D)
C_VIEW = (4, 8 * 1024, DC)
C_BUF = (8, 5, 8 * 128, DC)
O_VIEW = (4, 2, 4 * D, M)
F_PIECES = M * F * 2 // 16384
O_GROUPS = ((0, D), (D, D), (2 * D, D), (3 * D, 32), (3 * D + 96, 32))
O_ROUNDS = ([(r, half) for r in (480, 496, *range(0, 160, 16)) for half in range(2)]
            + [(r + d, half) for r in range(160, 416, 64) for half in range(2) for d in range(0, 64, 16)])
O_LAST = ([(a, 416, 64) for a in (6, 4, 3, 7, 0, 5)] + [(2, 416, 32), (2, 448, 32)]
          + [(1, 416, 16), (1, 432, 16), (1, 448, 16), (1, 464, 8), (1, 472, 8)])
S_WQ, S_WUK, S_WUV, S_W1, S_W2, S_X, S_B1, S_B2, S_C0, S_C1 = range(10)
S_C2, S_C3, S_O = S_C1 + 8, S_C1 + 16, S_C1 + 24
S_LAST = S_O + len(O_GROUPS)


def _loop(lo, hi, body):
    lax.fori_loop(lo, hi, lambda i, _: body(i), None)


def _rows16(row):
    return pl.ds(row if isinstance(row, int) else pl.multiple_of(row, 16), 16)


def _rows8(v):
    return jnp.concatenate([v[:, j * 128:(j + 1) * 128] for j in range(M // 128)], axis=0)


def _kernel(x_hbm, ckv_hbm, wq_hbm, wuk_hbm, wuv_hbm, wo_hbm, w1_hbm, b1_hbm, w2_hbm, b2_hbm,
            o_hbm,
            x_buf, b1_buf, b2_buf, c_buf, wq_buf, wuk_buf, wuv_buf, wo_buf, w1_buf, w2_buf,
            xs, t8, qa_ref, acc_ref, m_ref, l_ref, a_buf, e_buf, ctx_ref, mul_ref, s_ref, o_buf, sems):
    def fetch(src, dst, sem, queue):
        pltpu.make_async_copy(src, dst, sems.at[sem]).start(priority=queue)

    def wait_filled(buf, sem):
        pltpu.make_async_copy(buf, buf, sems.at[sem]).wait()

    def w_run(hbm, buf, sem, a):
        return lambda j, queue: fetch(hbm.at[a, pl.ds(j * 2, 2)], buf.at[a, pl.ds(j * 2, 2)], sem, queue)

    def c_run(a, n, sem):
        def run(j, queue):
            fetch(ckv_hbm.at[pl.ds(a // 8, n), _rows16(a % 8 * 1024 + j * 16)],
                  c_buf.at[j >> 3, pl.ds((a + 5) // 8, n), _rows16((a + 5) % 8 * 128 + (j & 7) * 16)],
                  sem if sem == S_C0 else sem + (j >> 3), queue)
        return run

    def f_run(hbm, buf, sem, first):
        def run(j, queue):
            p = first + j
            exists = p >= 0 if first < 0 else first + 64 <= F_PIECES or p < F_PIECES
            pl.when(exists)(lambda: fetch(hbm.at[p], buf.at[p], sem, queue))
        return run

    w1_run = functools.partial(f_run, w1_hbm, w1_buf, S_W1)
    w2_run = functools.partial(f_run, w2_hbm, w2_buf, S_W2)
    first = ([w1_run(48)] + [w_run(wuv_hbm, wuv_buf, S_WUV, a) for a in range(4)]
             + [w_run(wuk_hbm, wuk_buf, S_WUK, a) for a in range(4)]
             + [w_run(wq_hbm, wq_buf, S_WQ, a) for a in range(4)] + [c_run(a, 1, S_C0) for a in range(3)])
    order = (0, 2, 4, 6, 1, 3, 5, 7)
    phases = (
        list(zip((0, 1, 0, 1, 1, 0, 1, 0, 1, 1, 0, 1, 0, 1, 1, 1), [first[i + k] for i in order for k in (0, 8)])),
        [(i // 2 % 2, c_run(3 + i, 2, S_C1)) for i in order],
        [(1, c_run(19, 2, S_C2)), (0, c_run(21, 2, S_C2)), (1, c_run(23, 2, S_C2)),
         (0, c_run(25, 1, S_C3)), (1, w2_run(33)), (0, c_run(20, 2, S_C2)), (1, c_run(22, 2, S_C2)),
         (1, c_run(24, 1, S_C3)), (0, w2_run(-31)), (1, c_run(26, 1, S_C3)), (0, w2_run(97)), (0, w1_run(-16))],
    )
    ones = [[run for queue, run in phase if queue] for phase in phases]

    def o_copy(queue, sem, mib, half, row, cols=pl.ds(0, M)):
        idx = (mib, half, row, cols)
        return queue, functools.partial(fetch, wo_hbm.at[idx], wo_buf.at[idx], sem, queue)

    o_list = [o_copy(queue, S_O + (row // D if row < 480 else 4), pl.ds(queue, 1 + 2 * queue), half, pl.ds(row, 16))
              for row, half in O_ROUNDS for queue in range(2)]
    for i, (a, row, rows) in enumerate(O_LAST):
        if rows == 64:
            o_list += [o_copy(0, S_LAST + i, a // 2, a % 2, pl.ds(row, 16)),
                       o_copy(1, S_LAST + i, a // 2, a % 2, pl.ds(row + 16, 48))]
        else:
            o_list += [o_copy(1, S_LAST + i, a // 2, a % 2, pl.ds(r, 8), pl.ds(c, 256))
                       for r in range(row, row + rows, 8) for c in (0, 256)]
    o_ones = [start for queue, start in o_list if queue]
    ahead = iter(o_ones[LEAD:])
    o_starts = [start for start in (next(ahead, None) if queue else start for queue, start in o_list) if start]

    def starts(v, j):
        out, k, n = [], LEAD, len(ones[v])
        for queue, run in phases[v]:
            if not queue:
                out.append(functools.partial(run, j, 0))
            elif not isinstance(j, int) or j + k // n < 64:
                out.append(functools.partial(ones[v][k % n], j + k // n, 1))
            elif v < 2:
                r, i = divmod((j - 64) * n + k, len(ones[v + 1]))
                out.append(functools.partial(ones[v + 1][i], r, 1))
            else:
                out.append(o_ones[(j - 64) * n + k])
            k += queue
        return out

    def issue(batch):
        for start in batch:
            start()

    inner = [64 - pl.cdiv(LEAD, len(o)) for o in ones]

    def issue_rounds(v, lo, hi):
        _loop(lo, hi, lambda j: issue(starts(v, j)))

    def issue_rest(v):
        for j in range(inner[v], 64):
            issue(starts(v, j))

    round0 = list(zip(phases[0], starts(0, 0)))
    for g in range(LEAD):
        ones[0][g % len(ones[0])](g // len(ones[0]), 1)
        if g % 12 == 0:
            round0.pop([queue for (queue, _), _ in round0].index(0))[1]()
    issue([start for _, start in round0] + starts(0, 1))
    fetch(x_hbm, x_buf, S_X, 0)
    fetch(b1_hbm, b1_buf, S_B1, 0)
    fetch(b2_hbm, b2_buf, S_B2, 0)
    issue_rounds(0, 2, 16)

    wait_filled(x_buf, S_X)
    x = x_buf[...].astype(F32)
    xc = x - jnp.mean(x, axis=-1, keepdims=True)
    var = jnp.mean(xc * xc, axis=-1, keepdims=True)
    xn = (xc * lax.rsqrt(var + 1e-5)).astype(BF16)
    xf = xn.astype(F32)
    for b in range(B):
        for j in range(M // 128):
            cols = slice(j * 128, (j + 1) * 128)
            xs[b, cols, :] = jnp.broadcast_to(xf[b:b + 1, cols], (128, 128)).T
    e_buf[...] = (lax.broadcasted_iota(jnp.int32, (128, 128 * HG), 1) // HG
                  == lax.broadcasted_iota(jnp.int32, (128, 128 * HG), 0)).astype(F32).astype(BF16)
    m_ref[...] = jnp.full((B * H, 128), -jnp.inf, F32)
    l_ref[...] = jnp.zeros((B * H, 128), F32)
    acc_ref[...] = jnp.zeros((B * H, DC), F32)
    s_ref[...] = _rows8(x)
    issue_rounds(0, 16, inner[0])
    issue_rest(0)
    issue_rounds(1, 0, 8)

    wait_filled(wq_buf, S_WQ)

    def q_run(a, carry):
        def q_body(i, carry):
            q0, q1 = carry
            for u in range(8):
                m = pl.ds(a * 128 + i * 8 + u, 1)
                w = wq_buf[a, i * 8 + u].astype(F32)
                q0 = q0 + xs[0, m, :] * w
                q1 = q1 + xs[1, m, :] * w
            return q0, q1

        carry = lax.fori_loop(0, 16, q_body, carry)
        issue_rounds(1, 8 + 2 * a, 10 + 2 * a)
        return carry

    q0, q1 = lax.fori_loop(0, 4, q_run, (jnp.zeros((H, D), F32), jnp.zeros((H, D), F32)))
    q = jnp.concatenate([q0, q1, jnp.zeros((128 - B * H, D), F32)], axis=0).astype(BF16)

    wait_filled(wuk_buf, S_WUK)
    group = (lax.broadcasted_iota(jnp.int32, (16, 8, 128), 2) % H) // 8

    def qa_run(a):
        for u in range(8):
            w = wuk_buf[a, pl.ds(u * 16, 16)].reshape(16 * H, D)
            r = lax.dot_general(w, q, NT, preferred_element_type=F32).reshape(16, 4, 8, 128)
            v = jnp.where(group == 0, r[:, 0],
                          jnp.where(group == 1, r[:, 1], jnp.where(group == 2, r[:, 2], r[:, 3])))
            t8[pl.ds(pl.multiple_of((a * 8 + u) * 128, 128), 128), :] = v.reshape(128, 128)
        issue_rounds(1, 16 + 3 * a, 19 + 3 * a)

    _loop(0, 4, qa_run)
    sub = lax.broadcasted_iota(jnp.int32, (128, 128), 1) % 8
    for j in range(DC // 128):
        t = t8[pl.ds(j * 1024, 128, stride=8), :]
        for s in range(1, 8):
            t = jnp.where(sub == s, t8[pl.ds(j * 1024 + s, 128, stride=8), :], t)
        qa_ref[:, j * 128:(j + 1) * 128] = (t.T[:B * H] * (D ** -0.5 * LOG2E)).astype(BF16)

    wait_filled(c_buf.at[:, 0, pl.ds(640, 384)], S_C0)
    wait_filled(wuv_buf, S_WUV)
    diag = (lax.broadcasted_iota(jnp.int32, (H, 128 * HG), 1) % HG
            == lax.broadcasted_iota(jnp.int32, (H, 128 * HG), 0) % HG)

    def started(i):
        return jnp.maximum(30 + 6 * i, 15 + 8 * i)

    def block(i):
        lo, hi = jnp.where(i == 8, started(7) + 4, jnp.maximum(started(i - 1), 28)), started(i)
        for v, v0 in ((1, 0), (2, 64)):
            issue_rounds(v, jnp.maximum(lo - v0, 0), jnp.minimum(hi - v0, inner[v]))
            pl.when(jnp.logical_and(lo < v0 + 62, hi >= v0 + 62))(lambda: issue_rest(v))
        pl.when(i == 15)(lambda: issue(o_starts[:60]))

        b, g = i >> 3, i & 7
        pl.when(b == 0)(lambda: wait_filled(c_buf.at[g, pl.ds(1, 2)], S_C1 + g))
        pl.when(b == 1)(lambda: wait_filled(c_buf.at[g, pl.ds(3, 2), pl.ds(0, 640)], S_C2 + g))
        pl.when(b == 1)(lambda: wait_filled(c_buf.at[g, 3, pl.ds(640, 384)], S_C3 + g))
        c = jnp.concatenate([c_buf[g, 2 * b, 640:], c_buf[g, 2 * b + 1], c_buf[g, 2 * b + 2, :640]], axis=0)
        hrows = pl.ds(pl.multiple_of(b * H, H), H)
        sc = lax.dot_general(qa_ref[hrows, :], c, NT, preferred_element_type=F32)
        m_prev = m_ref[hrows, :]
        m_new = jnp.maximum(m_prev, jnp.max(sc, axis=1, keepdims=True))
        p = jnp.exp2(sc - m_new[:, :1])
        alpha = jnp.exp2(m_prev - m_new)
        l_ref[hrows, :] = alpha * l_ref[hrows, :] + jnp.sum(p, axis=1, keepdims=True)
        m_ref[hrows, :] = m_new
        pv = jnp.dot(p.astype(BF16), c, preferred_element_type=F32)
        acc_ref[hrows, :] = acc_ref[hrows, :] * alpha[:, :1] + pv

        @pl.when(g == 7)
        def _():
            pl.when(b == 0)(lambda: issue_rounds(2, hi - 64, hi - 60))
            pl.when(b == 1)(lambda: issue(o_starts[60:100]))
            pc = (acc_ref[hrows, :] / l_ref[hrows, :][:, :1]).astype(BF16)
            pc = jnp.concatenate([pc[:, j * 128:(j + 1) * 128] for j in range(DC // 128)], axis=0)
            rep = jnp.dot(pc, e_buf[...], preferred_element_type=F32)
            for j in range(DC // 128):
                a = jnp.where(diag, rep[j * H:(j + 1) * H], 0.0).astype(BF16)
                for k in range(H // HG):
                    a_buf[k, j, b] = a[k * HG:(k + 1) * HG]

        @pl.when(i == 15)
        def _():
            for k in range(H // HG):
                ctx = sum(jnp.dot(a_buf[k, j].reshape(B * HG, 128 * HG),
                                  wuv_buf[j, :, k * HG:(k + 1) * HG].reshape(128 * HG, D),
                                  preferred_element_type=F32) for j in range(DC // 128))
                for r in range(B):
                    ctx_ref[r * H + k * HG:r * H + (k + 1) * HG] = ctx[r * HG:(r + 1) * HG]

    _loop(0, 16, block)
    issue(o_starts[100:])

    wait_filled(w1_buf, S_W1)
    wait_filled(w2_buf, S_W2)
    wait_filled(b1_buf, S_B1)
    wait_filled(b2_buf, S_B2)
    w1 = w1_buf[...].reshape(M // 8, F // 128, 8, 128)
    hid = jnp.concatenate([jnp.dot(xn, w1[:, n].reshape(M, 128), preferred_element_type=F32)
                           for n in range(F // 128)], axis=1)
    hid = jax.nn.gelu(hid + b1_buf[...].astype(F32).reshape(1, F), approximate=True).astype(BF16)
    z = jnp.dot(hid, w2_buf[...].reshape(F, M), preferred_element_type=F32)
    z8 = _rows8(z + b2_buf[...].astype(F32).reshape(1, M))
    g8 = z8 * jax.nn.sigmoid(z8)

    odd = lax.broadcasted_iota(jnp.int32, (1, D), 1) % 2 == 1
    for a in range(H // 4):
        c0, c1 = (ctx_ref[pl.ds(b * H + 4 * a + 3, 1), :].astype(BF16).astype(F32) for b in range(B))
        mul_ref[0, a] = jnp.broadcast_to(jnp.where(odd, c1, c0), (128, D)).T
        mul_ref[1, a] = jnp.broadcast_to(jnp.where(odd, c0, c1), (128, D)).T

    def wait_group(g):
        wait_filled(wo_buf.at[:, :, pl.ds(*O_GROUPS[g])], S_O + g)

    def project(lo, hi):
        lhs = jnp.concatenate([ctx_ref[pl.ds(h, B, stride=H), :] for h in range(H) if lo <= h % 4 < hi], axis=1)
        rhs = wo_buf[:, :, lo * D:hi * D].reshape(8 * (hi - lo) * D, M)
        s_ref[...] += _rows8(jnp.dot(lhs.astype(BF16), rhs, preferred_element_type=F32)) * g8

    part = [[None] * (M // 128) for _ in range(2)]

    def accumulate(a, row, rows):
        for r in range(row, row + rows, 8):
            w = wo_buf[a // 2, a % 2, r:r + 8].astype(F32)
            for e in range(2):
                mul = mul_ref[e, a, r - 3 * D:r - 3 * D + 8]
                for j in range(M // 128):
                    t = w[:, j * 128:(j + 1) * 128] * mul
                    part[e][j] = t if part[e][j] is None else part[e][j] + t

    for g in (4, 0, 1):
        wait_group(g)
    project(0, 2)
    for a in range(8):
        accumulate(a, *O_GROUPS[4])
    wait_group(2)
    project(2, 3)
    base8 = s_ref[...]
    wait_group(3)
    for a in range(8):
        accumulate(a, *O_GROUPS[3])
    for i, (a, row, rows) in enumerate(O_LAST):
        wait_filled(wo_buf.at[a // 2, a % 2, pl.ds(row, rows)], S_LAST + i)
        accumulate(a, row, rows)

    sl = lax.broadcasted_iota(jnp.int32, (8, 128), 0)

    def merge(lo, hi, k):
        m = (sl & k) != 0
        return jnp.where(m, hi, lo), pltpu.roll(jnp.where(m, lo, hi), k, 0)

    r1 = [part[0][j] + pltpu.roll(part[1][j], 1, 0) for j in range(4)]
    r2 = [jnp.add(*merge(r1[j], r1[j + 1], 2)) for j in (0, 2)]
    near, far = merge(r2[0], r2[1], 4)
    o_buf[...] = (base8 + g8 * near + g8 * far).astype(BF16)
    store = pltpu.make_async_copy(o_buf, o_hbm, sems.at[S_X])
    store.start()
    store.wait()


@jax.jit
def pallas_recurrent_scan__compressed_kv_cla__dense_activation_gelu__decode_kernel(
    A_x: jax.Array,
    A_c_kv: jax.Array,
    A_w_q: jax.Array,
    A_w_uk: jax.Array,
    A_w_uv: jax.Array,
    A_w_o: jax.Array,
    B_x: jax.Array,
    B_w1: jax.Array,
    B_b1: jax.Array,
    B_w2: jax.Array,
    B_b2: jax.Array,
):
    del B_x
    hbm = pl.BlockSpec(memory_space=pltpu.HBM)
    w1_view, w2_view = (F_PIECES, 64, 128), (F_PIECES, 16, M)
    w1 = B_w1.reshape(M // 8, 8, F // 128, 128).transpose(0, 2, 1, 3).reshape(w1_view)
    out = pl.pallas_call(
        _kernel,
        out_shape=jax.ShapeDtypeStruct((8, 128), BF16),
        in_specs=[hbm] * 10,
        out_specs=hbm,
        scratch_shapes=[
            pltpu.VMEM((B, M), BF16), pltpu.VMEM((F,), BF16), pltpu.VMEM((M,), BF16),
            pltpu.VMEM(C_BUF, BF16), pltpu.VMEM(W_VIEW, BF16), pltpu.VMEM(W_VIEW, BF16),
            pltpu.VMEM(W_VIEW, BF16), pltpu.VMEM(O_VIEW, BF16),
            pltpu.VMEM(w1_view, BF16), pltpu.VMEM(w2_view, BF16),
            pltpu.VMEM((B, M, 128), F32),
            pltpu.VMEM((DC * 8 + 8, 128), F32),
            pltpu.VMEM((B * H, DC), BF16), pltpu.VMEM((B * H, DC), F32),
            pltpu.VMEM((B * H, 128), F32), pltpu.VMEM((B * H, 128), F32),
            pltpu.VMEM((H // HG, DC // 128, B, HG, 128 * HG), BF16), pltpu.VMEM((128, 128 * HG), BF16),
            pltpu.VMEM((3 * H, D), F32), pltpu.VMEM((B, H // 4, D, 128), F32),
            pltpu.VMEM((8, 128), F32), pltpu.VMEM((8, 128), BF16),
            pltpu.SemaphoreType.DMA((S_LAST + len(O_LAST),)),
        ],
        compiler_params=pltpu.CompilerParams(
            vmem_limit_bytes=100 * 1024 * 1024, disable_semaphore_checks=True, disable_bounds_checks=True),
    )(A_x.reshape(B, M), A_c_kv.reshape(C_VIEW), A_w_q.reshape(W_VIEW), A_w_uk.reshape(W_VIEW),
      A_w_uv.reshape(W_VIEW), A_w_o.reshape(O_VIEW), w1, B_b1, B_w2.reshape(w2_view), B_b2)
    return out.reshape(M // 128, B, 128).transpose(1, 0, 2).reshape(B, 1, M)
```

```python
import functools

import jax
import jax.numpy as jnp
from jax import lax
import jax.experimental.pallas as pl
import jax.experimental.pallas.tpu as pltpu

F32 = jnp.float32
BF16 = jnp.bfloat16

B, H, SK, D, M, DC, F = 2, 32, 16384, 128, 512, 512, 1792
LOG2E = 1.4426950408889634
NT = (((1,), (1,)), ((), ()))
HG = 16

LEAD = 26
W_VIEW = (4, 128, H, D)
C_VIEW = (4, 8, 64, 16, DC)
C_BUF = (5, 8, 64, 16, DC)
O_VIEW = (4, 2, 4 * D, M)
F_PIECES = M * F * 2 // 16384
O_GROUPS = ((0, D), (D, D), (2 * D, D), (3 * D, 32), (3 * D + 96, 32))
O_ROUNDS = ([(r, half) for r in (480, 496, *range(0, 160, 16)) for half in range(2)]
            + [(r + d, half) for r in range(160, 416, 64) for half in range(2) for d in range(0, 64, 16)])
O_LAST = ([(a, 416, 64) for a in (6, 4, 3, 7, 0, 5)] + [(2, 416, 32), (2, 448, 32)]
          + [(1, r, 8) for r in range(416, 480, 8)])
S_WQ, S_WUK, S_WUV, S_W1, S_W2, S_X, S_B1, S_B2, S_C0, S_C1 = range(10)
S_C2, S_C3, S_O = S_C1 + 8, S_C1 + 16, S_C1 + 24
S_LAST = S_O + len(O_GROUPS)


def _loop(lo, hi, body):
    lax.fori_loop(lo, hi, lambda i, _: body(i), None)


def _rows8(v):
    return jnp.concatenate([v[:, j * 128:(j + 1) * 128] for j in range(M // 128)], axis=0)


def _kernel(x_hbm, ckv_hbm, wq_hbm, wuk_hbm, wuv_hbm, wo_hbm, w1_hbm, b1_hbm, w2_hbm, b2_hbm,
            o_hbm,
            x_buf, b1_buf, b2_buf, c_buf, wq_buf, wuk_buf, wuv_buf, wo_buf, w1_buf, w2_buf,
            xs, t8, qa_ref, acc_ref, m_ref, l_ref, a_buf, e_buf, ctx_ref, mul_ref, s_ref, o_buf, sems):
    def fetch(src, dst, sem, queue):
        pltpu.make_async_copy(src, dst, sems.at[sem]).start(priority=queue)

    def wait_filled(buf, sem):
        pltpu.make_async_copy(buf, buf, sems.at[sem]).wait()

    def w_run(hbm, buf, sem, a):
        return lambda j, queue: fetch(hbm.at[a, pl.ds(j * 2, 2)], buf.at[a, pl.ds(j * 2, 2)], sem, queue)

    def c_run(a, n, sem):
        return lambda j, queue: fetch(
            ckv_hbm.at[pl.ds(a // 8, n), a % 8, j], c_buf.at[pl.ds((a + 5) // 8, n), (a + 5) % 8, j],
            sem if sem == S_C0 else sem + (j >> 3), queue)

    def f_run(hbm, buf, sem, first):
        def run(j, queue):
            p = first + j
            exists = p >= 0 if first < 0 else first + 64 <= F_PIECES or p < F_PIECES
            pl.when(exists)(lambda: fetch(hbm.at[p], buf.at[p], sem, queue))
        return run

    w1_run = functools.partial(f_run, w1_hbm, w1_buf, S_W1)
    w2_run = functools.partial(f_run, w2_hbm, w2_buf, S_W2)
    first = ([w1_run(48)] + [w_run(wuv_hbm, wuv_buf, S_WUV, a) for a in range(4)]
             + [w_run(wuk_hbm, wuk_buf, S_WUK, a) for a in range(4)]
             + [w_run(wq_hbm, wq_buf, S_WQ, a) for a in range(4)] + [c_run(a, 1, S_C0) for a in range(3)])
    order = (0, 2, 4, 6, 1, 3, 5, 7)
    phases = (
        list(zip((0, 1, 0, 1, 1, 0, 1, 0, 1, 1, 0, 1, 0, 1, 1, 1), [first[i + k] for i in order for k in (0, 8)])),
        [(i // 2 % 2, c_run(3 + i, 2, S_C1)) for i in order],
        [(1, c_run(19, 2, S_C2)), (1, c_run(21, 2, S_C2)), (0, c_run(26, 1, S_C3)), (1, c_run(24, 1, S_C3)),
         (0, c_run(23, 2, S_C2)), (1, c_run(25, 1, S_C3)), (0, c_run(20, 2, S_C2)), (1, w2_run(33)),
         (1, c_run(22, 2, S_C2)), (0, w2_run(-31)), (0, w2_run(97)), (0, w1_run(-16))],
    )
    ones = [[run for queue, run in phase if queue] for phase in phases]

    def o_copy(queue, sem, mib, half, row, cols=pl.ds(0, M)):
        idx = (mib, half, row, cols)
        return queue, functools.partial(fetch, wo_hbm.at[idx], wo_buf.at[idx], sem, queue)

    o_list = [o_copy(queue, S_O + (row // D if row < 480 else 4), pl.ds(queue, 1 + 2 * queue), half, pl.ds(row, 16))
              for row, half in O_ROUNDS for queue in range(2)]
    for i, (a, row, rows) in enumerate(O_LAST):
        if rows == 64:
            o_list += [o_copy(0, S_LAST + i, a // 2, a % 2, pl.ds(row, 16)),
                       o_copy(1, S_LAST + i, a // 2, a % 2, pl.ds(row + 16, 48))]
        else:
            o_list += [o_copy(1, S_LAST + i, a // 2, a % 2, pl.ds(r, 8), pl.ds(c, 256))
                       for r in range(row, row + rows, 8) for c in (0, 256)]
    o_ones = [start for queue, start in o_list if queue]
    ahead = iter(o_ones[LEAD:])
    o_starts = [start for start in (next(ahead, None) if queue else start for queue, start in o_list) if start]

    def starts(v, j):
        out, k, n = [], LEAD, len(ones[v])
        for queue, run in phases[v]:
            if not queue:
                out.append(functools.partial(run, j, 0))
            elif not isinstance(j, int) or j + k // n < 64:
                out.append(functools.partial(ones[v][k % n], j + k // n, 1))
            elif v < 2:
                r, i = divmod((j - 64) * n + k, len(ones[v + 1]))
                out.append(functools.partial(ones[v + 1][i], r, 1))
            else:
                out.append(o_ones[(j - 64) * n + k])
            k += queue
        return out

    def issue(batch):
        for start in batch:
            start()

    inner = [64 - pl.cdiv(LEAD, len(o)) for o in ones]

    def issue_rounds(v, lo, hi):
        _loop(lo, hi, lambda j: issue(starts(v, j)))

    def issue_rest(v):
        for j in range(inner[v], 64):
            issue(starts(v, j))

    round0 = list(zip(phases[0], starts(0, 0)))
    for g in range(LEAD):
        ones[0][g % len(ones[0])](g // len(ones[0]), 1)
        if g % 9 == 0:
            round0.pop([queue for (queue, _), _ in round0].index(0))[1]()
    issue([start for _, start in round0] + starts(0, 1))
    fetch(x_hbm, x_buf, S_X, 0)
    fetch(b1_hbm, b1_buf, S_B1, 0)
    fetch(b2_hbm, b2_buf, S_B2, 0)
    issue_rounds(0, 2, 16)

    wait_filled(x_buf, S_X)
    x = x_buf[...].astype(F32)
    xc = x - jnp.mean(x, axis=-1, keepdims=True)
    var = jnp.mean(xc * xc, axis=-1, keepdims=True)
    xn = (xc * lax.rsqrt(var + 1e-5)).astype(BF16)
    xf = xn.astype(F32)
    for b in range(B):
        for j in range(M // 128):
            cols = slice(j * 128, (j + 1) * 128)
            xs[b, cols, :] = jnp.broadcast_to(xf[b:b + 1, cols], (128, 128)).T
    e_buf[...] = (lax.broadcasted_iota(jnp.int32, (128, 128 * HG), 1) // HG
                  == lax.broadcasted_iota(jnp.int32, (128, 128 * HG), 0)).astype(F32).astype(BF16)
    m_ref[...] = jnp.full((B * H, 128), -jnp.inf, F32)
    l_ref[...] = jnp.zeros((B * H, 128), F32)
    acc_ref[...] = jnp.zeros((B * H, DC), F32)
    s_ref[...] = _rows8(x)
    issue_rounds(0, 16, inner[0])
    issue_rest(0)
    issue_rounds(1, 0, 8)

    wait_filled(wq_buf, S_WQ)

    def q_run(a, carry):
        def q_body(i, carry):
            q0, q1 = carry
            for u in range(8):
                m = pl.ds(a * 128 + i * 8 + u, 1)
                w = wq_buf[a, i * 8 + u].astype(F32)
                q0 = q0 + xs[0, m, :] * w
                q1 = q1 + xs[1, m, :] * w
            return q0, q1

        carry = lax.fori_loop(0, 16, q_body, carry)
        issue_rounds(1, 8 + 2 * a, 10 + 2 * a)
        return carry

    q0, q1 = lax.fori_loop(0, 4, q_run, (jnp.zeros((H, D), F32), jnp.zeros((H, D), F32)))
    q = jnp.concatenate([q0, q1, jnp.zeros((128 - B * H, D), F32)], axis=0).astype(BF16)

    wait_filled(wuk_buf, S_WUK)
    group = (lax.broadcasted_iota(jnp.int32, (16, 8, 128), 2) % H) // 8

    def qa_run(a):
        for u in range(8):
            w = wuk_buf[a, pl.ds(u * 16, 16)].reshape(16 * H, D)
            r = lax.dot_general(w, q, NT, preferred_element_type=F32).reshape(16, 4, 8, 128)
            v = jnp.where(group == 0, r[:, 0],
                          jnp.where(group == 1, r[:, 1], jnp.where(group == 2, r[:, 2], r[:, 3])))
            t8[pl.ds(pl.multiple_of((a * 8 + u) * 128, 128), 128), :] = v.reshape(128, 128)
        issue_rounds(1, 16 + 3 * a, 19 + 3 * a)

    _loop(0, 4, qa_run)
    sub = lax.broadcasted_iota(jnp.int32, (128, 128), 1) % 8
    for j in range(DC // 128):
        t = t8[pl.ds(j * 1024, 128, stride=8), :]
        for s in range(1, 8):
            t = jnp.where(sub == s, t8[pl.ds(j * 1024 + s, 128, stride=8), :], t)
        qa_ref[:, j * 128:(j + 1) * 128] = (t.T[:B * H] * (D ** -0.5 * LOG2E)).astype(BF16)

    wait_filled(c_buf.at[0, pl.ds(5, 3)], S_C0)
    wait_filled(wuv_buf, S_WUV)
    diag = (lax.broadcasted_iota(jnp.int32, (H, 128 * HG), 1) % HG
            == lax.broadcasted_iota(jnp.int32, (H, 128 * HG), 0) % HG)

    def started(i):
        return jnp.maximum(30 + 6 * i, 15 + 8 * i)

    def block(i):
        lo, hi = jnp.where(i == 8, started(7) + 4, jnp.maximum(started(i - 1), 28)), started(i)
        for v, v0 in ((1, 0), (2, 64)):
            issue_rounds(v, jnp.clip(lo - v0, 0, inner[v]), jnp.clip(hi - v0, 0, inner[v]))
            pl.when(jnp.logical_and(lo < v0 + 62, hi >= v0 + 62))(lambda: issue_rest(v))
        pl.when(i == 15)(lambda: issue(o_starts[:60]))

        b, g = i >> 3, i & 7
        js = pl.ds(g * 8, 8)
        pl.when(b == 0)(lambda: wait_filled(c_buf.at[pl.ds(1, 2), :, js], S_C1 + g))
        pl.when(b == 1)(lambda: wait_filled(c_buf.at[pl.ds(3, 2), pl.ds(0, 5), js], S_C2 + g))
        pl.when(b == 1)(lambda: wait_filled(c_buf.at[3, pl.ds(5, 3), js], S_C3 + g))
        c = jnp.concatenate([c_buf[2 * b, 5:, js], c_buf[2 * b + 1, :, js], c_buf[2 * b + 2, :5, js]],
                            axis=0).reshape(16 * 128, DC)
        hrows = pl.ds(pl.multiple_of(b * H, H), H)
        sc = lax.dot_general(qa_ref[hrows, :], c, NT, preferred_element_type=F32)
        m_prev = m_ref[hrows, :]
        m_new = jnp.maximum(m_prev, jnp.max(sc, axis=1, keepdims=True))
        p = jnp.exp2(sc - m_new[:, :1])
        alpha = jnp.exp2(m_prev - m_new)
        l_ref[hrows, :] = alpha * l_ref[hrows, :] + jnp.sum(p, axis=1, keepdims=True)
        m_ref[hrows, :] = m_new
        pv = jnp.dot(p.astype(BF16), c, preferred_element_type=F32)
        acc_ref[hrows, :] = acc_ref[hrows, :] * alpha[:, :1] + pv

        @pl.when(g == 7)
        def _():
            pl.when(b == 0)(lambda: issue_rounds(2, hi - 64, hi - 60))
            pl.when(b == 1)(lambda: issue(o_starts[60:100]))
            pc = (acc_ref[hrows, :] / l_ref[hrows, :][:, :1]).astype(BF16)
            pc = jnp.concatenate([pc[:, j * 128:(j + 1) * 128] for j in range(DC // 128)], axis=0)
            rep = jnp.dot(pc, e_buf[...], preferred_element_type=F32)
            for j in range(DC // 128):
                a = jnp.where(diag, rep[j * H:(j + 1) * H], 0.0).astype(BF16)
                for k in range(H // HG):
                    a_buf[k, j, b] = a[k * HG:(k + 1) * HG]

        @pl.when(i == 15)
        def _():
            for k in range(H // HG):
                ctx = sum(jnp.dot(a_buf[k, j].reshape(B * HG, 128 * HG),
                                  wuv_buf[j, :, k * HG:(k + 1) * HG].reshape(128 * HG, D),
                                  preferred_element_type=F32) for j in range(DC // 128))
                for r in range(B):
                    ctx_ref[r * H + k * HG:r * H + (k + 1) * HG] = ctx[r * HG:(r + 1) * HG]

    _loop(0, 16, block)
    issue(o_starts[100:])

    wait_filled(w1_buf, S_W1)
    wait_filled(w2_buf, S_W2)
    wait_filled(b1_buf, S_B1)
    wait_filled(b2_buf, S_B2)
    w1 = w1_buf[...].reshape(M // 8, F // 128, 8, 128)
    hid = jnp.concatenate([jnp.dot(xn, w1[:, n].reshape(M, 128), preferred_element_type=F32)
                           for n in range(F // 128)], axis=1)
    hid = jax.nn.gelu(hid + b1_buf[...].astype(F32).reshape(1, F), approximate=True).astype(BF16)
    z = jnp.dot(hid, w2_buf[...].reshape(F, M), preferred_element_type=F32)
    z8 = _rows8(z + b2_buf[...].astype(F32).reshape(1, M))
    g8 = z8 * jax.nn.sigmoid(z8)

    odd = lax.broadcasted_iota(jnp.int32, (1, D), 1) % 2 == 1
    for a in range(H // 4):
        c0, c1 = (ctx_ref[pl.ds(b * H + 4 * a + 3, 1), :].astype(BF16).astype(F32) for b in range(B))
        mul_ref[0, a] = jnp.broadcast_to(jnp.where(odd, c1, c0), (128, D)).T
        mul_ref[1, a] = jnp.broadcast_to(jnp.where(odd, c0, c1), (128, D)).T

    def wait_group(g):
        wait_filled(wo_buf.at[:, :, pl.ds(*O_GROUPS[g])], S_O + g)

    def project(lo, hi):
        lhs = jnp.concatenate([ctx_ref[pl.ds(h, B, stride=H), :] for h in range(H) if lo <= h % 4 < hi], axis=1)
        rhs = wo_buf[:, :, lo * D:hi * D].reshape(8 * (hi - lo) * D, M)
        s_ref[...] += _rows8(jnp.dot(lhs.astype(BF16), rhs, preferred_element_type=F32)) * g8

    part = [[None] * (M // 128) for _ in range(2)]

    def accumulate(a, row, rows):
        for r in range(row, row + rows, 8):
            w = wo_buf[a // 2, a % 2, r:r + 8].astype(F32)
            for e in range(2):
                mul = mul_ref[e, a, r - 3 * D:r - 3 * D + 8]
                for j in range(M // 128):
                    t = w[:, j * 128:(j + 1) * 128] * mul
                    part[e][j] = t if part[e][j] is None else part[e][j] + t

    for g in (4, 0, 1):
        wait_group(g)
    project(0, 2)
    for a in range(8):
        accumulate(a, *O_GROUPS[4])
    wait_group(2)
    project(2, 3)
    base8 = s_ref[...]
    wait_group(3)
    for a in range(8):
        accumulate(a, *O_GROUPS[3])
    for i, (a, row, rows) in enumerate(O_LAST):
        wait_filled(wo_buf.at[a // 2, a % 2, pl.ds(row, rows)], S_LAST + i)
        accumulate(a, row, rows)

    sl = lax.broadcasted_iota(jnp.int32, (8, 128), 0)

    def merge(lo, hi, k):
        m = (sl & k) != 0
        return jnp.where(m, hi, lo), pltpu.roll(jnp.where(m, lo, hi), k, 0)

    r1 = [part[0][j] + pltpu.roll(part[1][j], 1, 0) for j in range(4)]
    r2 = [jnp.add(*merge(r1[j], r1[j + 1], 2)) for j in (0, 2)]
    near, far = merge(r2[0], r2[1], 4)
    o_buf[...] = (base8 + g8 * near + g8 * far).astype(BF16)
    store = pltpu.make_async_copy(o_buf, o_hbm, sems.at[S_X])
    store.start()
    store.wait()


@jax.jit
def pallas_recurrent_scan__compressed_kv_cla__dense_activation_gelu__decode_kernel(
    A_x: jax.Array,
    A_c_kv: jax.Array,
    A_w_q: jax.Array,
    A_w_uk: jax.Array,
    A_w_uv: jax.Array,
    A_w_o: jax.Array,
    B_x: jax.Array,
    B_w1: jax.Array,
    B_b1: jax.Array,
    B_w2: jax.Array,
    B_b2: jax.Array,
):
    del B_x
    hbm = pl.BlockSpec(memory_space=pltpu.HBM)
    w1_view, w2_view = (F_PIECES, 64, 128), (F_PIECES, 16, M)
    w1 = B_w1.reshape(M // 8, 8, F // 128, 128).transpose(0, 2, 1, 3).reshape(w1_view)
    out = pl.pallas_call(
        _kernel,
        out_shape=jax.ShapeDtypeStruct((8, 128), BF16),
        in_specs=[hbm] * 10,
        out_specs=hbm,
        scratch_shapes=[
            pltpu.VMEM((B, M), BF16), pltpu.VMEM((F,), BF16), pltpu.VMEM((M,), BF16),
            pltpu.VMEM(C_BUF, BF16), pltpu.VMEM(W_VIEW, BF16), pltpu.VMEM(W_VIEW, BF16),
            pltpu.VMEM(W_VIEW, BF16), pltpu.VMEM(O_VIEW, BF16),
            pltpu.VMEM(w1_view, BF16), pltpu.VMEM(w2_view, BF16),
            pltpu.VMEM((B, M, 128), F32),
            pltpu.VMEM((DC * 8 + 8, 128), F32),
            pltpu.VMEM((B * H, DC), BF16), pltpu.VMEM((B * H, DC), F32),
            pltpu.VMEM((B * H, 128), F32), pltpu.VMEM((B * H, 128), F32),
            pltpu.VMEM((H // HG, DC // 128, B, HG, 128 * HG), BF16), pltpu.VMEM((128, 128 * HG), BF16),
            pltpu.VMEM((3 * H, D), F32), pltpu.VMEM((B, H // 4, D, 128), F32),
            pltpu.VMEM((8, 128), F32), pltpu.VMEM((8, 128), BF16),
            pltpu.SemaphoreType.DMA((S_LAST + len(O_LAST),)),
        ],
        compiler_params=pltpu.CompilerParams(
            vmem_limit_bytes=100 * 1024 * 1024, disable_semaphore_checks=True, disable_bounds_checks=True),
    )(A_x.reshape(B, M), A_c_kv.reshape(C_VIEW), A_w_q.reshape(W_VIEW), A_w_uk.reshape(W_VIEW),
      A_w_uv.reshape(W_VIEW), A_w_o.reshape(O_VIEW), w1, B_b1, B_w2.reshape(w2_view), B_b2)
    return out.reshape(M // 128, B, 128).transpose(1, 0, 2).reshape(B, 1, M)
```
